```python
import jax
import jax.numpy as jnp

def _softmax(x, axis=-1):
    return jax.nn.softmax(x, axis=axis)
def _gelu(x):
    return jax.nn.gelu(x, approximate=True)
def _silu(x):
    return jax.nn.silu(x)
def _sigmoid(x):
    return jax.nn.sigmoid(x)
def _layernorm(x, axis=-1, eps=1e-5):
    m = jnp.mean(x, axis=axis, keepdims=True)
    v = jnp.var(x, axis=axis, keepdims=True)
    return (x - m) / jnp.sqrt(v + eps)
def _scatter_add(tgt, idx, src, axis=0):
    return tgt.at[idx].add(src)
def _segment_sum(src, seg, n):
    return jax.ops.segment_sum(src, seg, n)
class _Rng:
    def __init__(self, key):
        self._k = key
    def _next(self):
        self._k, sub = jax.random.split(self._k)
        return sub
    def normal(self, shape):
        return jax.random.normal(self._next(), shape, dtype=jnp.bfloat16)
    def randint(self, lo, hi, shape):
        return jax.random.randint(self._next(), shape, lo, hi, dtype=jnp.int32)
    def uniform(self, shape, lo=0.0, hi=1.0):
        return jax.random.uniform(self._next(), shape, jnp.bfloat16, lo, hi)
    def permutation(self, n):
        return jax.random.permutation(self._next(), n)


kernel_name = 'sequential_preLN__sliding_block_cached__mixer_s_mlp__decode'

def setup_inputs():
    _rng = _Rng(jax.random.key(int.from_bytes(__import__("os").urandom(4), "little")))
    _w = (lambda a: (lambda t: t.astype(jnp.bfloat16) if jnp.issubdtype(t.dtype, jnp.floating) else t)(jnp.asarray(a)))
    def _A_setup():
        B, Sq, D = 1, 1, 640
        Hq, Hkv, Sk, Dh = 32, 32, 32768, 192
        assert Hq % Hkv == 0, (Hq, Hkv)
        return {
            "x": _w((lambda *s: _rng.normal(s) * 0.05)(B, Sq, D)),
            "k_cache": _w((lambda *s: _rng.normal(s) * 0.05)(B, Hkv, Sk, Dh)),
            "v_cache": _w((lambda *s: _rng.normal(s) * 0.05)(B, Hkv, Sk, Dh)),
            "wq": _w((lambda *s: _rng.normal(s) * 0.05)(D, Hq * Dh) * (D ** -0.5)),
            "wo": _w((lambda *s: _rng.normal(s) * 0.05)(Hq * Dh, D) * ((Hq * Dh) ** -0.5)),
        }
    _A_in = _A_setup()

    def _B_setup():
        B, S, D, F = 1, 1, 640, 1536
        return {
            "x":  _w((lambda *s: _rng.normal(s) * 0.05)(B, S, D)),
            "w1": _w((lambda *s: _rng.normal(s) * 0.05)(D, D) * (D ** -0.5)),
            "w2": _w((lambda *s: _rng.normal(s) * 0.05)(D, D) * (D ** -0.5)),
            "w3": _w((lambda *s: _rng.normal(s) * 0.05)(D, F) * (D ** -0.5)),
            "w4": _w((lambda *s: _rng.normal(s) * 0.05)(F, D) * (F ** -0.5)),
        }
    _B_in = _B_setup()

    return {
        "A_x": _A_in["x"],
        "A_k_cache": _A_in["k_cache"],
        "A_v_cache": _A_in["v_cache"],
        "A_wq": _A_in["wq"],
        "A_wo": _A_in["wo"],
        "B_x": _B_in["x"],
        "B_w1": _B_in["w1"],
        "B_w2": _B_in["w2"],
        "B_w3": _B_in["w3"],
        "B_w4": _B_in["w4"],
    }

def reference(A_x, A_k_cache, A_v_cache, A_wq, A_wo, B_x, B_w1, B_w2, B_w3, B_w4):
    def _A_ref(x, k_cache, v_cache, wq, wo):
        B, Sq, D = x.shape
        Hq, Dh = 32, 192
        Hkv, Sk = k_cache.shape[1], k_cache.shape[2]
        W = min(4096, max(256, Sk // 4))
        rep = Hq // Hkv
        q = (lambda x, *d: x.transpose(*d))((x @ wq).reshape(B, Sq, Hq, Dh), 0, 2, 1, 3)
        k = jnp.repeat(k_cache[:, :, Sk - W:, :], rep, axis=1)
        v = jnp.repeat(v_cache[:, :, Sk - W:, :], rep, axis=1)
        scores = jnp.einsum("bhqd,bhkd->bhqk", q, k) * (Dh ** -0.5)
        p = _softmax(scores, axis=-1)
        o = jnp.einsum("bhqk,bhkd->bhqd", p, v)
        return (lambda x, *d: x.transpose(*d))(o, 0, 2, 1, 3).reshape(B, Sq, Hq * Dh) @ wo

    def _B_ref(x, w1, w2, w3, w4):
        B, S, D = x.shape
        h = _gelu(_layernorm(x, axis=-1) @ w1)
        c = D // 4
        g0 = jnp.pad(h[:, :, 0*c:1*c], ((0, 0), (1, 0), (0, 0)))[:, :S, :]
        g1 = jnp.pad(h[:, :, 1*c:2*c], ((0, 0), (0, 1), (0, 0)))[:, 1:, :]
        g2 = jnp.pad(h[:, :, 2*c:3*c], ((0, 0), (2, 0), (0, 0)))[:, :S, :]
        g3 = jnp.pad(h[:, :, 3*c:   ], ((0, 0), (0, 2), (0, 0)))[:, 2:, :]
        hs = jnp.concatenate([g0, g1, g2, g3], axis=-1) @ w2
        x1 = x + hs
        h2 = _gelu(_layernorm(x1, axis=-1) @ w3) @ w4
        return x1 + h2

    x = A_x
    h = x + _A_ref(_layernorm(x, axis=-1), A_k_cache, A_v_cache, A_wq, A_wo)
    h2 = h + _B_ref(_layernorm(h, axis=-1), B_w1, B_w2, B_w3, B_w4)
    return h2
```

```python
import jax
import jax.numpy as jnp
import jax.experimental.pallas as pl
import jax.experimental.pallas.tpu as pltpu

D = 640
HQ = 32
DH = 192
F = 1536
EPS = 1e-5
NPAIR = HQ // 2
PR = 2 * DH


def _ln(v):
    m = jnp.mean(v, axis=-1, keepdims=True)
    c = v - m
    var = jnp.mean(c * c, axis=-1, keepdims=True)
    return c * jax.lax.rsqrt(var + EPS)


def make(NS=2, W4C=4, name="decode_v1"):
    def kernel(x_hbm, k_hbm, v_hbm, wq_hbm, wo_hbm, w3_hbm, w4_hbm, o_ref,
               x_buf, wq_buf, k_buf, v_buf, wo_buf, w3_buf, w4_buf,
               sem_x, sem_wq, sem_k, sem_v, sem_wo, sem_w3, sem_w4):
        S = k_hbm.shape[1]
        W = min(4096, max(256, S // 4))
        scale = DH ** -0.5

        def cp_wq(j, slot):
            c0 = pl.multiple_of(j * PR, 128)
            return pltpu.make_async_copy(wq_hbm.at[:, pl.ds(c0, PR)], wq_buf.at[slot], sem_wq.at[slot])

        def cp_k(j, slot):
            r0 = pl.multiple_of(j * PR, PR)
            return pltpu.make_async_copy(k_hbm.at[pl.ds(r0, PR), pl.ds(S - W, W)], k_buf.at[slot], sem_k.at[slot])

        def cp_v(j, slot):
            r0 = pl.multiple_of(j * PR, PR)
            return pltpu.make_async_copy(v_hbm.at[pl.ds(r0, PR), pl.ds(S - W, W)], v_buf.at[slot], sem_v.at[slot])

        def cp_wo(j, slot):
            r0 = pl.multiple_of(j * PR, PR)
            return pltpu.make_async_copy(wo_hbm.at[pl.ds(r0, PR), :], wo_buf.at[slot], sem_wo.at[slot])

        cp_x = pltpu.make_async_copy(x_hbm, x_buf, sem_x.at[0])
        cp_w3 = pltpu.make_async_copy(w3_hbm, w3_buf, sem_w3.at[0])
        R4 = F // W4C

        def cp_w4(c):
            return pltpu.make_async_copy(w4_hbm.at[pl.ds(c * R4, R4), :], w4_buf.at[pl.ds(c * R4, R4), :], sem_w4.at[c])

        cp_x.start()
        for j in range(NS):
            cp_wq(j, j).start()
            cp_k(j, j).start()
            cp_v(j, j).start()
            cp_wo(j, j).start()

        cp_x.wait()
        x8 = jnp.broadcast_to(x_buf[...].astype(jnp.float32), (8, D))
        xln = _ln(x8).astype(jnp.bfloat16)

        row = jax.lax.broadcasted_iota(jnp.int32, (8, PR), 0)
        col = jax.lax.broadcasted_iota(jnp.int32, (8, PR), 1)
        mask = ((row == 0) & (col < DH)) | ((row == 1) & (col >= DH))

        def body(j, acc):
            slot = j % NS
            jn = jnp.minimum(j + NS, NPAIR - 1)
            more = j + NS < NPAIR
            cp_wq(j, slot).wait()
            q = jnp.dot(xln, wq_buf[slot], preferred_element_type=jnp.float32)
            qbd = jnp.where(mask, q, 0.0).astype(jnp.bfloat16)

            @pl.when(more)
            def _():
                cp_wq(jn, slot).start()

            cp_k(j, slot).wait()
            s = jnp.dot(qbd, k_buf[slot], preferred_element_type=jnp.float32) * scale

            @pl.when(more)
            def _():
                cp_k(jn, slot).start()

            m = jnp.max(s, axis=-1, keepdims=True)
            p = jnp.exp(s - m)
            l = jnp.sum(p, axis=-1, keepdims=True)
            pb = p.astype(jnp.bfloat16)
            cp_v(j, slot).wait()
            o = jax.lax.dot_general(pb, v_buf[slot], (((1,), (1,)), ((), ())), preferred_element_type=jnp.float32)

            @pl.when(more)
            def _():
                cp_v(jn, slot).start()

            obd = jnp.where(mask, o / l, 0.0).astype(jnp.bfloat16)
            cp_wo(j, slot).wait()
            acc = acc + jnp.dot(obd, wo_buf[slot], preferred_element_type=jnp.float32)

            @pl.when(more)
            def _():
                cp_wo(jn, slot).start()

            @pl.when(j == NPAIR - 1 - NS)
            def _():
                cp_w3.start()
                for c in range(W4C):
                    cp_w4(c).start()

            return acc

        acc = jax.lax.fori_loop(0, NPAIR, body, jnp.zeros((8, D), jnp.float32))
        attn = jnp.sum(acc, axis=0, keepdims=True)
        h = x8 + jnp.broadcast_to(attn, (8, D))
        xb = _ln(h)
        x2 = _ln(xb).astype(jnp.bfloat16)
        cp_w3.wait()
        a = jnp.dot(x2, w3_buf[...], preferred_element_type=jnp.float32)
        g = jax.nn.gelu(a, approximate=True).astype(jnp.bfloat16)
        y = h + xb
        for c in range(W4C):
            cp_w4(c).wait()
            y = y + jnp.dot(g[:, c * R4:(c + 1) * R4], w4_buf[pl.ds(c * R4, R4), :], preferred_element_type=jnp.float32)
        o_ref[...] = y[0:1, :].astype(o_ref.dtype)

    def f(A_x, A_k_cache, A_v_cache, A_wq, A_wo, B_x, B_w1, B_w2, B_w3, B_w4):
        B, Hkv, Sk, Dh = A_k_cache.shape
        kt = jnp.swapaxes(A_k_cache, 2, 3).reshape(Hkv * Dh, Sk)
        vt = jnp.swapaxes(A_v_cache, 2, 3).reshape(Hkv * Dh, Sk)
        x = A_x.reshape(1, D)
        W = min(4096, max(256, Sk // 4))
        any_spec = pl.BlockSpec(memory_space=pl.ANY)
        out = pl.pallas_call(
            kernel,
            out_shape=jax.ShapeDtypeStruct((1, D), jnp.bfloat16),
            in_specs=[any_spec] * 7,
            out_specs=pl.BlockSpec(memory_space=pltpu.VMEM),
            scratch_shapes=[
                pltpu.VMEM((1, D), jnp.bfloat16),
                pltpu.VMEM((NS, D, PR), jnp.bfloat16),
                pltpu.VMEM((NS, PR, W), jnp.bfloat16),
                pltpu.VMEM((NS, PR, W), jnp.bfloat16),
                pltpu.VMEM((NS, PR, D), jnp.bfloat16),
                pltpu.VMEM((D, F), jnp.bfloat16),
                pltpu.VMEM((F, D), jnp.bfloat16),
                pltpu.SemaphoreType.DMA((1,)),
                pltpu.SemaphoreType.DMA((NS,)),
                pltpu.SemaphoreType.DMA((NS,)),
                pltpu.SemaphoreType.DMA((NS,)),
                pltpu.SemaphoreType.DMA((NS,)),
                pltpu.SemaphoreType.DMA((1,)),
                pltpu.SemaphoreType.DMA((W4C,)),
            ],
            compiler_params=pltpu.CompilerParams(vmem_limit_bytes=64 * 1024 * 1024),
            name=name,
        )(x, kt, vt, A_wq, A_wo, B_w3, B_w4)
        return out.reshape(1, 1, D)

    return f


_impl = make(2, 4, name="preln_decode_fused")


@jax.jit
def pallas_sequential_preLN__sliding_block_cached__mixer_s_mlp__decode_kernel(
    A_x: jax.Array,
    A_k_cache: jax.Array,
    A_v_cache: jax.Array,
    A_wq: jax.Array,
    A_wo: jax.Array,
    B_x: jax.Array,
    B_w1: jax.Array,
    B_w2: jax.Array,
    B_w3: jax.Array,
    B_w4: jax.Array,
):
    return _impl(A_x, A_k_cache, A_v_cache, A_wq, A_wo, B_x, B_w1, B_w2, B_w3, B_w4)
```

```python
import contextlib
import jax
import jax.numpy as jnp
import jax.experimental.pallas as pl
import jax.experimental.pallas.tpu as pltpu

D = 640
HQ = 32
DH = 192
F = 1536
EPS = 1e-5
NPAIR = HQ // 2
PR = 2 * DH


def _ln(v):
    m = jnp.mean(v, axis=-1, keepdims=True)
    c = v - m
    var = jnp.mean(c * c, axis=-1, keepdims=True)
    return c * jax.lax.rsqrt(var + EPS)


def _cut(total, pattern):
    out, r, i = [], 0, 0
    while r < total:
        n, pr = pattern[i % len(pattern)]
        n = min(n, total - r)
        out.append((r, n, pr)); r += n; i += 1
    return out


def make(N=8, pkv=((8, 0), (24, 1)), pwq=((80, 0), (240, 1)), pwo=((48, 0), (144, 1)), pw3=((32, 0), (96, 1)),
         pw4=((64, 0), (192, 1)), skeleton=False, name="decode_v4", scopes=False, NQ=4, extra=None,
         w3_cols=2, w4_rows=128, tail_per_step=1):
    extra = extra or {}

    def sc(n):
        return jax.named_scope(n) if scopes else contextlib.nullcontext()

    pair_chunks = ([("wq",) + c for c in _cut(D, pwq)] + [("k",) + c for c in _cut(PR, pkv)] +
                   [("v",) + c for c in _cut(PR, pkv)] + [("wo",) + c for c in _cut(PR, pwo)])
    tail_chunks = [("w3",) + c for c in _cut(D, pw3)] + [("w4",) + c for c in _cut(F, pw4)]
    C = len(pair_chunks)
    CT = len(tail_chunks)
    NSEM = N

    def ready_step(chunks, kind, row_end):
        for i, (k, r, n, pr) in enumerate(chunks):
            if k == kind and r + n >= row_end:
                return i
        raise ValueError

    pieces = [("q", ready_step(pair_chunks, "wq", D))]
    for b in range(3):
        for c in range(NQ):
            pieces.append((("qk", b, c), ready_step(pair_chunks, "k", 128 * (b + 1))))
    pieces.append((("sm", 0), 0))
    pieces.append((("sm", 1), 0))
    for b in range(3):
        for c in range(NQ):
            pieces.append((("pv", b, c), ready_step(pair_chunks, "v", 128 * (b + 1))))
    pieces.append((("wo",), ready_step(pair_chunks, "wo", PR)))
    pieces[0] = (("q",), pieces[0][1])
    NP = len(pieces)
    slot_step = [((i + 1) * C) // NP - 1 for i in range(NP)]
    table = None
    for shift in range(NP):
        ok = True
        tb = {}
        for i, (pc, rdy) in enumerate(pieces):
            s = i + shift
            if s < NP and slot_step[s] < rdy:
                ok = False
                break
            tb.setdefault(slot_step[s % NP], []).append((pc, s >= NP))
        if ok:
            table = tb
            break
    assert table is not None
    make.last_table = (shift, table)

    def kernel(x_hbm, k_hbm, v_hbm, wq_hbm, wo_hbm, w3_hbm, w4_hbm, o_ref,
               x_buf, wq_buf, k_buf, v_buf, wo_buf, w3_buf, w4_buf, p_buf, sem_x, sem_p):
        S = k_hbm.shape[1]
        W = min(4096, max(256, S // 4))
        WQ = W // NQ
        scale = DH ** -0.5

        def cp_pair(j, c):
            kind, r, n, pr = pair_chunks[c]
            slot = j % 2
            base = j * PR
            if not isinstance(j, int):
                base = pl.multiple_of(base, PR)
            if kind == "wq":
                src = wq_hbm.at[pl.ds(r, n), pl.ds(base, PR)]
                dst = wq_buf.at[slot, pl.ds(r, n)]
            elif kind == "k":
                src = k_hbm.at[pl.ds(base + r, n), pl.ds(S - W, W)]
                dst = k_buf.at[slot, pl.ds(r, n)]
            elif kind == "v":
                src = v_hbm.at[pl.ds(base + r, n), pl.ds(S - W, W)]
                dst = v_buf.at[slot, pl.ds(r, n)]
            else:
                src = wo_hbm.at[pl.ds(base + r, n), :]
                dst = wo_buf.at[slot, pl.ds(r, n)]
            if C % NSEM == 0:
                si = c % NSEM
            else:
                si = (j * C + c) % NSEM
            return pltpu.make_async_copy(src, dst, sem_p.at[si]), pr

        def cp_tail(c):
            kind, r, n, pr = tail_chunks[c]
            if kind == "w3":
                src, dst = w3_hbm.at[pl.ds(r, n), :], w3_buf.at[pl.ds(r, n), :]
            else:
                src, dst = w4_hbm.at[pl.ds(r, n), :], w4_buf.at[pl.ds(r, n), :]
            return pltpu.make_async_copy(src, dst, sem_p.at[(NPAIR * C + c) % NSEM]), pr

        def start(cp):
            cp[0].start(priority=cp[1])

        cp_x = pltpu.make_async_copy(x_hbm, x_buf, sem_x.at[0])
        cp_x.start()
        for c in range(N):
            start(cp_pair(0, c))
        cp_x.wait()
        x8 = jnp.broadcast_to(x_buf[...].astype(jnp.float32), (8, D))
        xln = _ln(x8).astype(jnp.bfloat16)

        row = jax.lax.broadcasted_iota(jnp.int32, (8, PR), 0)
        col = jax.lax.broadcasted_iota(jnp.int32, (8, PR), 1)
        mask = ((row == 0) & (col < DH)) | ((row == 1) & (col >= DH))

        def run_piece(pc, j, st):
            slot = j % 2
            if pc[0] == "q":
                q = jnp.dot(xln, wq_buf[slot], preferred_element_type=jnp.float32)
                st["qbd"] = jnp.where(mask, q, 0.0).astype(jnp.bfloat16)
            elif pc[0] == "qk":
                _, b, c = pc
                part = jnp.dot(st["qbd"][:, b * 128:(b + 1) * 128], k_buf[slot, pl.ds(b * 128, 128), pl.ds(c * WQ, WQ)],
                               preferred_element_type=jnp.float32)
                st[("s", c)] = part if b == 0 else st[("s", c)] + part
            elif pc[0] == "sm":
                if pc[1] == 0:
                    for c in range(NQ):
                        st[("s", c)] = st[("s", c)] * scale
                    m = st[("s", 0)]
                    for c in range(1, NQ):
                        m = jnp.maximum(m, st[("s", c)])
                    st["m"] = jnp.max(m, axis=-1, keepdims=True)
                    cs = range(0, NQ // 2)
                    st["lsum"] = None
                else:
                    cs = range(NQ // 2, NQ)
                for c in cs:
                    p = jnp.exp(st[("s", c)] - st["m"])
                    st["lsum"] = p if st["lsum"] is None else st["lsum"] + p
                    p_buf[:, pl.ds(c * WQ, WQ)] = p.astype(jnp.bfloat16)
                if pc[1] == 1:
                    st["l"] = jnp.sum(st["lsum"], axis=-1, keepdims=True)
            elif pc[0] == "pv":
                _, b, c = pc
                o_t = jax.lax.dot_general(p_buf[:, pl.ds(c * WQ, WQ)], v_buf[slot, pl.ds(b * 128, 128), pl.ds(c * WQ, WQ)],
                                          (((1,), (1,)), ((), ())), preferred_element_type=jnp.float32)
                st[("o", b)] = o_t if c == 0 else st[("o", b)] + o_t
            elif pc[0] == "wo":
                o = jnp.concatenate([st[("o", b)] for b in range(3)], axis=1)
                obd = jnp.where(mask, o / st["l"], 0.0).astype(jnp.bfloat16)
                st["acc"] = st["acc"] + jnp.dot(obd, wo_buf[slot], preferred_element_type=jnp.float32)

        carried = [pc for stp in sorted(table) for pc, prev in table[stp] if prev]
        carry_keys = ["acc", "l"] + [("o", b) for b in range(3)]
        assert all(pc[0] in ("pv", "wo") for pc in carried), carried

        def pair_body(j, st, first, last):
            prev = dict(st)
            cur = {"acc": st["acc"]}
            for c in range(C):
                cp_pair(j, c)[0].wait()
                nx = c + N
                if nx < C:
                    start(cp_pair(j, nx))
                elif not last:
                    start(cp_pair(j + 1, nx - C))
                elif nx - C < CT:
                    start(cp_tail(nx - C))
                if skeleton:
                    continue
                for pc, is_prev in table.get(c, []):
                    if is_prev:
                        if not first:
                            prev["acc"] = cur["acc"]
                            run_piece(pc, j - 1, prev)
                            cur["acc"] = prev["acc"]
                    else:
                        run_piece(pc, j, cur)
            return cur

        z = jnp.zeros((8, D), jnp.float32)
        if skeleton:
            def lb(j, a):
                pair_body(j, {"acc": a}, False, False)
                return a
            pair_body(0, {"acc": z}, True, False)
            jax.lax.fori_loop(1, NPAIR - 1, lb, z)
            st = pair_body(NPAIR - 1, {"acc": z}, False, True)
            st["acc"] = z
        else:
            st = pair_body(0, {"acc": z}, True, False)
            init = tuple(st[k] for k in carry_keys)

            def lb(j, carry):
                s_in = dict(zip(carry_keys, carry))
                s_out = pair_body(j, s_in, False, False)
                return tuple(s_out[k] for k in carry_keys)

            carry = jax.lax.fori_loop(1, NPAIR - 1, lb, init)
            st = pair_body(NPAIR - 1, dict(zip(carry_keys, carry)), False, True)

        tail_pieces = [(pc, 0) for pc in carried]
        tail_pieces.append((("ln",), 0))
        W3C = F // w3_cols
        for b in range(D // 128):
            for cc in range(w3_cols):
                tail_pieces.append((("w3", b, cc), ready_step(tail_chunks, "w3", 128 * (b + 1))))
        tail_pieces.append((("gelu",), 0))
        for b in range(F // w4_rows):
            tail_pieces.append((("w4", b), ready_step(tail_chunks, "w4", w4_rows * (b + 1))))
        tp = 0

        def run_tail(pc):
            if pc[0] == "ln":
                attn = jnp.sum(st["acc"], axis=0, keepdims=True)
                h = x8 + jnp.broadcast_to(attn, (8, D))
                xb = _ln(h)
                st["x2"] = _ln(xb).astype(jnp.bfloat16)
                st["y"] = h + xb
            elif pc[0] == "w3":
                _, b, cc = pc
                part = jnp.dot(st["x2"][:, b * 128:(b + 1) * 128], w3_buf[pl.ds(b * 128, 128), pl.ds(cc * W3C, W3C)],
                               preferred_element_type=jnp.float32)
                st[("a", cc)] = part if b == 0 else st[("a", cc)] + part
            elif pc[0] == "gelu":
                a = jnp.concatenate([st[("a", cc)] for cc in range(w3_cols)], axis=1)
                st["g"] = jax.nn.gelu(a, approximate=True).astype(jnp.bfloat16)
            elif pc[0] == "w4":
                b = pc[1]
                st["y"] = st["y"] + jnp.dot(st["g"][:, b * w4_rows:(b + 1) * w4_rows], w4_buf[pl.ds(b * w4_rows, w4_rows), :],
                                            preferred_element_type=jnp.float32)
            else:
                run_piece(pc, NPAIR - 1, st)

        for c in range(CT):
            with sc(f"t_{tail_chunks[c][0]}_{tail_chunks[c][1] + tail_chunks[c][2]}"):
                cp_tail(c)[0].wait()
            if c + N < CT:
                start(cp_tail(c + N))
            if skeleton:
                continue
            budget = tail_per_step if c < CT - 1 else 10 ** 6
            while tp < len(tail_pieces) and budget > 0 and tail_pieces[tp][1] <= c:
                run_tail(tail_pieces[tp][0])
                tp += 1
                budget -= 1
        if skeleton:
            st["y"] = x8
        with sc("final_store"):
            o_ref[...] = st["y"][0:1, :].astype(o_ref.dtype)

    def f(A_x, A_k_cache, A_v_cache, A_wq, A_wo, B_x, B_w1, B_w2, B_w3, B_w4):
        B, Hkv, Sk, Dh = A_k_cache.shape
        kt = jnp.swapaxes(A_k_cache, 2, 3).reshape(Hkv * Dh, Sk)
        vt = jnp.swapaxes(A_v_cache, 2, 3).reshape(Hkv * Dh, Sk)
        x = A_x.reshape(1, D)
        W = min(4096, max(256, Sk // 4))
        any_spec = pl.BlockSpec(memory_space=pl.ANY)
        out = pl.pallas_call(
            kernel,
            out_shape=jax.ShapeDtypeStruct((1, D), jnp.bfloat16),
            in_specs=[any_spec] * 7,
            out_specs=pl.BlockSpec(memory_space=pltpu.VMEM),
            scratch_shapes=[
                pltpu.VMEM((1, D), jnp.bfloat16),
                pltpu.VMEM((2, D, PR), jnp.bfloat16),
                pltpu.VMEM((2, PR, W), jnp.bfloat16),
                pltpu.VMEM((2, PR, W), jnp.bfloat16),
                pltpu.VMEM((2, PR, D), jnp.bfloat16),
                pltpu.VMEM((D, F), jnp.bfloat16),
                pltpu.VMEM((F, D), jnp.bfloat16),
                pltpu.VMEM((8, W), jnp.bfloat16),
                pltpu.SemaphoreType.DMA((1,)),
                pltpu.SemaphoreType.DMA((NSEM,)),
            ],
            compiler_params=pltpu.CompilerParams(vmem_limit_bytes=64 * 1024 * 1024, **extra),
            name=name,
        )(x, kt, vt, A_wq, A_wo, B_w3, B_w4)
        return out.reshape(1, 1, D)

    f.__name__ = name
    return f


_impl = make(N=8, name="preln_decode_fused")


@jax.jit
def pallas_sequential_preLN__sliding_block_cached__mixer_s_mlp__decode_kernel(
    A_x: jax.Array,
    A_k_cache: jax.Array,
    A_v_cache: jax.Array,
    A_wq: jax.Array,
    A_wo: jax.Array,
    B_x: jax.Array,
    B_w1: jax.Array,
    B_w2: jax.Array,
    B_w3: jax.Array,
    B_w4: jax.Array,
):
    return _impl(A_x, A_k_cache, A_v_cache, A_wq, A_wo, B_x, B_w1, B_w2, B_w3, B_w4)
```

```python
import contextlib
import jax
import jax.numpy as jnp
import jax.experimental.pallas as pl
import jax.experimental.pallas.tpu as pltpu

D = 640
HQ = 32
DH = 192
F = 1536
EPS = 1e-5
NPAIR = HQ // 2
PR = 2 * DH
ROWB = {"wq": PR * 2, "k": 4096 * 2, "v": 4096 * 2, "wo": D * 2, "w3": F * 2, "w4": D * 2}


def _ln(v):
    m = jnp.mean(v, axis=-1, keepdims=True)
    c = v - m
    var = jnp.mean(c * c, axis=-1, keepdims=True)
    return c * jax.lax.rsqrt(var + EPS)


def _cut(total, pattern):
    out, r, i = [], 0, 0
    while r < total:
        e = pattern[i % len(pattern)]
        n, pr = e[0], e[1]
        ns = e[2] if len(e) > 2 else 1
        n = min(n, total - r)
        for s in range(ns):
            out.append((r, n, pr, s, ns))
        r += n; i += 1
    return out


def _patlen(pattern):
    return sum((e[2] if len(e) > 2 else 1) for e in pattern)


def _nbytes(c):
    return c[2] * ROWB[c[0]] // c[5]


def _merge(chunks, mode):
    if mode == "seq":
        return chunks
    q = [[c for c in chunks if c[3] == t] for t in (0, 1)]
    tot = [sum(_nbytes(c) for c in q[t]) for t in (0, 1)]
    keyed = []
    for t in (0, 1):
        acc = 0
        for c in q[t]:
            b = _nbytes(c)
            keyed.append(((acc + b * mode_off(mode, t)) / tot[t], t, len(keyed), c))
            acc += b
    keyed.sort()
    return [c for _, _, _, c in keyed]


def mode_off(mode, t):
    return {"prop": 1.0, "prop0": 0.0, "prop5": 0.5}[mode]


def make(LA=(4, 4), pkv=((8, 0), (8, 0), (8, 0), (24, 1)), pwq=((320, 1),), pwo=((192, 1),),
         pw3=((24, 0), (24, 0), (16, 0), (64, 1)), pw4=((48, 0), (48, 0), (32, 0), (128, 1)),
         merge="prop", tmerge="prop", skeleton=False, name="decode_v5", scopes=False, NQ=4, extra=None,
         w3_cols=2, w4_rows=128, tail_spread=True, place="bytes", poff=0, tpoff=0, pslots=None, wslots=None, tslots=None, fill=False):
    extra = extra or {}

    def sc(n):
        return jax.named_scope(n) if scopes else contextlib.nullcontext()

    pair_chunks = _merge([("wq",) + c for c in _cut(D, pwq)] + [("k",) + c for c in _cut(PR, pkv)] +
                         [("v",) + c for c in _cut(PR, pkv)] + [("wo",) + c for c in _cut(PR, pwo)], merge)
    tail_chunks = _merge([("w3",) + c for c in _cut(D, pw3)] + [("w4",) + c for c in _cut(F, pw4)], tmerge)
    C = len(pair_chunks)
    CT = len(tail_chunks)
    pq = [[i for i, c in enumerate(pair_chunks) if c[3] == t] for t in (0, 1)]
    tq = [[i for i, c in enumerate(tail_chunks) if c[3] == t] for t in (0, 1)]
    ppos = {i: k for t in (0, 1) for k, i in enumerate(pq[t])}
    tpos = {i: k for t in (0, 1) for k, i in enumerate(tq[t])}
    NQ0 = [len(pq[0]), len(pq[1])]
    assert all(NQ0[t] >= LA[t] for t in (0, 1)), NQ0
    SOFF = (0, LA[0])
    NSEM = LA[0] + LA[1]

    def ready_step(chunks, kind, row_end):
        return max(i for i, c in enumerate(chunks) if c[0] == kind and c[1] < row_end)

    pieces = [(("q",), ready_step(pair_chunks, "wq", D))]
    for b in range(3):
        for c in range(NQ):
            pieces.append((("qk", b, c), ready_step(pair_chunks, "k", 128 * (b + 1))))
    pieces.append((("sm", 0), 0))
    pieces.append((("sm", 1), 0))
    for b in range(3):
        for c in range(NQ):
            pieces.append((("pv", b, c), ready_step(pair_chunks, "v", 128 * (b + 1))))
    pieces.append((("wo",), ready_step(pair_chunks, "wo", PR)))
    NP = len(pieces)
    cum, tot = [], 0
    for c in pair_chunks:
        tot += _nbytes(c)
        cum.append(tot)
    if place == "bytes":
        slot_step = [min(i for i in range(C) if cum[i] >= (s + 1) * tot / NP - 1e-6) for s in range(NP)]
    elif place == "steps":
        slot_step = [((i + 1) * C) // NP - 1 for i in range(NP)]
    elif place == "q1":
        q1steps = pq[1]
        slot_step = [q1steps[min(len(q1steps) - 1, ((s + 1) * len(q1steps)) // NP - 1 if (s + 1) * len(q1steps) >= NP else 0)] for s in range(NP)]
    if place != "pat":
        slot_step = [max(0, min(C - 1, s + poff)) for s in slot_step]
    if place == "pat":
        cand = []
        cnt = {}
        for i, c in enumerate(pair_chunks):
            kind = c[0]
            k = cnt.get(kind, 0); cnt[kind] = k + 1
            if kind in ("k", "v"):
                L = _patlen(pkv)
                cand += [i] * list(pslots).count(k % L)
            else:
                L = _patlen(pwq if kind == "wq" else pwo)
                cand += [i] * list(wslots).count(k % L)
        if fill:
            slot_step = cand
        else:
            slot_step = [cand[(k * len(cand)) // NP] for k in range(NP)]
    if fill and place == "pat":
        nfill = len(slot_step) - NP
        newp, used = [], 0
        for i, pcs in enumerate(pieces):
            newp.append(pcs)
            want = ((i + 1) * nfill) // NP
            while used < want:
                newp.append((("dummy",), 0)); used += 1
        pieces = newp
        NP = len(pieces)
    table = None
    for shift in range(NP):
        ok = True
        tb = {}
        for i, (pc, rdy) in enumerate(pieces):
            s = i + shift
            if s < NP and slot_step[s] < rdy:
                ok = False
                break
            tb.setdefault(slot_step[s % NP], []).append((pc, s >= NP))
        if ok:
            table = tb
            break
    assert table is not None
    make.last = dict(shift=shift, table=table, C=C, CT=CT, NQ0=NQ0, pair=pair_chunks, tail=tail_chunks)

    def kernel(x_hbm, k_hbm, v_hbm, wq_hbm, wo_hbm, w3_hbm, w4_hbm, o_ref,
               x_buf, wq_buf, k_buf, v_buf, wo_buf, w3_buf, w4_buf, p_buf, sem_x, sem_p):
        S = k_hbm.shape[1]
        W = min(4096, max(256, S // 4))
        WQ = W // NQ
        scale = DH ** -0.5

        def cp_pair(j, c):
            kind, r, n, pr, cs, ns = pair_chunks[c]
            assert ns == 1 or kind in ("k", "v")
            cw = W // ns
            slot = j % 2
            base = j * PR
            if not isinstance(j, int):
                base = pl.multiple_of(base, PR)
            if kind == "wq":
                src = wq_hbm.at[pl.ds(r, n), pl.ds(base, PR)]
                dst = wq_buf.at[slot, pl.ds(r, n)]
            elif kind == "k":
                src = k_hbm.at[pl.ds(base + r, n), pl.ds(S - W + cs * cw, cw)]
                dst = k_buf.at[slot, pl.ds(r, n), pl.ds(cs * cw, cw)]
            elif kind == "v":
                src = v_hbm.at[pl.ds(base + r, n), pl.ds(S - W + cs * cw, cw)]
                dst = v_buf.at[slot, pl.ds(r, n), pl.ds(cs * cw, cw)]
            else:
                src = wo_hbm.at[pl.ds(base + r, n), :]
                dst = wo_buf.at[slot, pl.ds(r, n)]
            if NQ0[pr] % LA[pr] == 0:
                si = ppos[c] % LA[pr]
            else:
                si = (j * NQ0[pr] + ppos[c]) % LA[pr]
            return pltpu.make_async_copy(src, dst, sem_p.at[SOFF[pr] + si]), pr

        def cp_tail(c):
            kind, r, n, pr, cs, ns = tail_chunks[c]
            assert ns == 1
            if kind == "w3":
                src, dst = w3_hbm.at[pl.ds(r, n), :], w3_buf.at[pl.ds(r, n), :]
            else:
                src, dst = w4_hbm.at[pl.ds(r, n), :], w4_buf.at[pl.ds(r, n), :]
            si = (NPAIR * NQ0[pr] + tpos[c]) % LA[pr]
            return pltpu.make_async_copy(src, dst, sem_p.at[SOFF[pr] + si]), pr

        def start(cp):
            cp[0].start(priority=cp[1])

        def start_ahead(j, c, last):
            pr = pair_chunks[c][3]
            k = ppos[c] + LA[pr]
            if k < NQ0[pr]:
                start(cp_pair(j, pq[pr][k]))
            elif not last:
                start(cp_pair(j + 1, pq[pr][k - NQ0[pr]]))
            elif k - NQ0[pr] < len(tq[pr]):
                start(cp_tail(tq[pr][k - NQ0[pr]]))

        cp_x = pltpu.make_async_copy(x_hbm, x_buf, sem_x.at[0])
        cp_x.start()
        for c in sorted(pq[0][:LA[0]] + pq[1][:LA[1]]):
            start(cp_pair(0, c))
        cp_x.wait()
        x8 = jnp.broadcast_to(x_buf[...].astype(jnp.float32), (8, D))
        xln = _ln(x8).astype(jnp.bfloat16)

        row = jax.lax.broadcasted_iota(jnp.int32, (8, PR), 0)
        col = jax.lax.broadcasted_iota(jnp.int32, (8, PR), 1)
        mask = ((row == 0) & (col < DH)) | ((row == 1) & (col >= DH))

        def run_piece(pc, j, st):
            slot = j % 2
            if pc[0] == "q":
                q = jnp.dot(xln, wq_buf[slot], preferred_element_type=jnp.float32)
                st["qbd"] = jnp.where(mask, q, 0.0).astype(jnp.bfloat16)
            elif pc[0] == "qk":
                _, b, c = pc
                part = jnp.dot(st["qbd"][:, b * 128:(b + 1) * 128], k_buf[slot, pl.ds(b * 128, 128), pl.ds(c * WQ, WQ)],
                               preferred_element_type=jnp.float32)
                st[("s", c)] = part if b == 0 else st[("s", c)] + part
            elif pc[0] == "sm":
                if pc[1] == 0:
                    for c in range(NQ):
                        st[("s", c)] = st[("s", c)] * scale
                    m = st[("s", 0)]
                    for c in range(1, NQ):
                        m = jnp.maximum(m, st[("s", c)])
                    st["m"] = jnp.max(m, axis=-1, keepdims=True)
                    cs = range(0, NQ // 2)
                    st["lsum"] = None
                else:
                    cs = range(NQ // 2, NQ)
                for c in cs:
                    p = jnp.exp(st[("s", c)] - st["m"])
                    st["lsum"] = p if st["lsum"] is None else st["lsum"] + p
                    p_buf[:, pl.ds(c * WQ, WQ)] = p.astype(jnp.bfloat16)
                if pc[1] == 1:
                    st["l"] = jnp.sum(st["lsum"], axis=-1, keepdims=True)
            elif pc[0] == "pv":
                _, b, c = pc
                o_t = jax.lax.dot_general(p_buf[:, pl.ds(c * WQ, WQ)], v_buf[slot, pl.ds(b * 128, 128), pl.ds(c * WQ, WQ)],
                                          (((1,), (1,)), ((), ())), preferred_element_type=jnp.float32)
                st[("o", b)] = o_t if c == 0 else st[("o", b)] + o_t
            elif pc[0] == "dummy":
                pass
            elif pc[0] == "wo":
                o = jnp.concatenate([st[("o", b)] for b in range(3)], axis=1)
                obd = jnp.where(mask, o / st["l"], 0.0).astype(jnp.bfloat16)
                st["acc"] = st["acc"] + jnp.dot(obd, wo_buf[slot], preferred_element_type=jnp.float32)

        carried = [pc for stp in sorted(table) for pc, prev in table[stp] if prev]
        carry_keys = ["acc", "l"] + [("o", b) for b in range(3) if ("pv", b, 0) not in carried]
        assert all(pc[0] in ("pv", "wo") for pc in carried), carried

        def pair_body(j, st, first, last):
            prev = dict(st)
            cur = {"acc": st["acc"]}
            for c in range(C):
                cp_pair(j, c)[0].wait()
                start_ahead(j, c, last)
                if skeleton:
                    continue
                for pc, is_prev in table.get(c, []):
                    if is_prev:
                        if not first:
                            prev["acc"] = cur["acc"]
                            run_piece(pc, j - 1, prev)
                            cur["acc"] = prev["acc"]
                    else:
                        run_piece(pc, j, cur)
            return cur

        z = jnp.zeros((8, D), jnp.float32)
        if skeleton:
            def lb(j, a):
                pair_body(j, {"acc": a}, False, False)
                return a
            pair_body(0, {"acc": z}, True, False)
            jax.lax.fori_loop(1, NPAIR - 1, lb, z)
            st = pair_body(NPAIR - 1, {"acc": z}, False, True)
            st["acc"] = z
        else:
            st = pair_body(0, {"acc": z}, True, False)
            init = tuple(st[k] for k in carry_keys)

            def lb(j, carry):
                s_in = dict(zip(carry_keys, carry))
                s_out = pair_body(j, s_in, False, False)
                return tuple(s_out[k] for k in carry_keys)

            carry = jax.lax.fori_loop(1, NPAIR - 1, lb, init)
            st = pair_body(NPAIR - 1, dict(zip(carry_keys, carry)), False, True)

        tail_pieces = [(pc, 0) for pc in carried]
        tail_pieces.append((("ln",), 0))
        W3C = F // w3_cols
        for b in range(D // 128):
            for cc in range(w3_cols):
                tail_pieces.append((("w3", b, cc), ready_step(tail_chunks, "w3", 128 * (b + 1))))
        tail_pieces.append((("gelu",), 0))
        for b in range(F // w4_rows):
            tail_pieces.append((("w4", b), ready_step(tail_chunks, "w4", w4_rows * (b + 1))))
        tp = 0

        def run_tail(pc):
            if pc[0] == "ln":
                attn = jnp.sum(st["acc"], axis=0, keepdims=True)
                h = x8 + jnp.broadcast_to(attn, (8, D))
                xb = _ln(h)
                st["x2"] = _ln(xb).astype(jnp.bfloat16)
                st["y"] = h + xb
            elif pc[0] == "w3":
                _, b, cc = pc
                part = jnp.dot(st["x2"][:, b * 128:(b + 1) * 128], w3_buf[pl.ds(b * 128, 128), pl.ds(cc * W3C, W3C)],
                               preferred_element_type=jnp.float32)
                st[("a", cc)] = part if b == 0 else st[("a", cc)] + part
            elif pc[0] == "gelu":
                a = jnp.concatenate([st[("a", cc)] for cc in range(w3_cols)], axis=1)
                st["g"] = jax.nn.gelu(a, approximate=True).astype(jnp.bfloat16)
            elif pc[0] == "w4":
                b = pc[1]
                st["y"] = st["y"] + jnp.dot(st["g"][:, b * w4_rows:(b + 1) * w4_rows], w4_buf[pl.ds(b * w4_rows, w4_rows), :],
                                            preferred_element_type=jnp.float32)
            else:
                run_piece(pc, NPAIR - 1, st)

        tcum, ttot = [], 0
        for c in tail_chunks:
            ttot += _nbytes(c)
            tcum.append(ttot)
        NTP = len(tail_pieces)
        for c in range(CT):
            with sc(f"t_{tail_chunks[c][0]}_{tail_chunks[c][1] + tail_chunks[c][2]}"):
                cp_tail(c)[0].wait()
            pr = tail_chunks[c][3]
            k = tpos[c] + LA[pr]
            if k < len(tq[pr]):
                start(cp_tail(tq[pr][k]))
            if skeleton:
                continue
            allowed = NTP if c == CT - 1 else int(NTP * tcum[c] / ttot + 1e-6) + (1 if tail_spread else 10 ** 6)
            while tp < NTP and tp < allowed and tail_pieces[tp][1] <= c:
                run_tail(tail_pieces[tp][0])
                tp += 1
        if skeleton:
            st["y"] = x8
        with sc("final_store"):
            o_ref[...] = st["y"][0:1, :].astype(o_ref.dtype)

    def f(A_x, A_k_cache, A_v_cache, A_wq, A_wo, B_x, B_w1, B_w2, B_w3, B_w4):
        B, Hkv, Sk, Dh = A_k_cache.shape
        kt = jnp.swapaxes(A_k_cache, 2, 3).reshape(Hkv * Dh, Sk)
        vt = jnp.swapaxes(A_v_cache, 2, 3).reshape(Hkv * Dh, Sk)
        x = A_x.reshape(1, D)
        W = min(4096, max(256, Sk // 4))
        any_spec = pl.BlockSpec(memory_space=pl.ANY)
        out = pl.pallas_call(
            kernel,
            out_shape=jax.ShapeDtypeStruct((1, D), jnp.bfloat16),
            in_specs=[any_spec] * 7,
            out_specs=pl.BlockSpec(memory_space=pltpu.VMEM),
            scratch_shapes=[
                pltpu.VMEM((1, D), jnp.bfloat16),
                pltpu.VMEM((2, D, PR), jnp.bfloat16),
                pltpu.VMEM((2, PR, W), jnp.bfloat16),
                pltpu.VMEM((2, PR, W), jnp.bfloat16),
                pltpu.VMEM((2, PR, D), jnp.bfloat16),
                pltpu.VMEM((D, F), jnp.bfloat16),
                pltpu.VMEM((F, D), jnp.bfloat16),
                pltpu.VMEM((8, W), jnp.bfloat16),
                pltpu.SemaphoreType.DMA((1,)),
                pltpu.SemaphoreType.DMA((NSEM,)),
            ],
            compiler_params=pltpu.CompilerParams(vmem_limit_bytes=64 * 1024 * 1024, **extra),
            name=name,
        )(x, kt, vt, A_wq, A_wo, B_w3, B_w4)
        return out.reshape(1, 1, D)

    f.__name__ = name
    return f


_impl = make(pkv=((8, 0, 4), (40, 1)), pwq=((80, 0), (240, 1)), pwo=((48, 0), (144, 1)), place="pat", NQ=8, pslots=(0, 1, 2), wslots=(0, 1), LA=(6, 4), pw3=((32, 0), (96, 1)), pw4=((64, 0), (192, 1)), merge="seq", tmerge="seq", name="preln_decode_fused")


@jax.jit
def pallas_sequential_preLN__sliding_block_cached__mixer_s_mlp__decode_kernel(
    A_x: jax.Array,
    A_k_cache: jax.Array,
    A_v_cache: jax.Array,
    A_wq: jax.Array,
    A_wo: jax.Array,
    B_x: jax.Array,
    B_w1: jax.Array,
    B_w2: jax.Array,
    B_w3: jax.Array,
    B_w4: jax.Array,
):
    return _impl(A_x, A_k_cache, A_v_cache, A_wq, A_wo, B_x, B_w1, B_w2, B_w3, B_w4)
```

```python
import contextlib
import jax
import jax.numpy as jnp
import jax.experimental.pallas as pl
import jax.experimental.pallas.tpu as pltpu

D = 640
HQ = 32
DH = 192
F = 1536
EPS = 1e-5
NPAIR = HQ // 2
PR = 2 * DH
ROWB = {"wq": PR * 2, "k": 4096 * 2, "v": 4096 * 2, "wo": D * 2, "w3": F * 2, "w4": D * 2}


def _ln(v):
    m = jnp.mean(v, axis=-1, keepdims=True)
    c = v - m
    var = jnp.mean(c * c, axis=-1, keepdims=True)
    return c * jax.lax.rsqrt(var + EPS)


def _cut(total, pattern):
    out, r, i = [], 0, 0
    while r < total:
        e = pattern[i % len(pattern)]
        n, pr = e[0], e[1]
        ns = e[2] if len(e) > 2 else 1
        n = min(n, total - r)
        for s in range(ns):
            out.append((r, n, pr, s, ns))
        r += n; i += 1
    return out


def _patlen(pattern):
    return sum((e[2] if len(e) > 2 else 1) for e in pattern)


def _nbytes(c):
    return c[2] * ROWB[c[0]] // c[5]


def _merge(chunks, mode):
    if mode == "seq":
        return chunks
    q = [[c for c in chunks if c[3] == t] for t in (0, 1)]
    tot = [sum(_nbytes(c) for c in q[t]) for t in (0, 1)]
    keyed = []
    for t in (0, 1):
        acc = 0
        for c in q[t]:
            b = _nbytes(c)
            keyed.append(((acc + b * mode_off(mode, t)) / tot[t], t, len(keyed), c))
            acc += b
    keyed.sort()
    return [c for _, _, _, c in keyed]


def mode_off(mode, t):
    return {"prop": 1.0, "prop0": 0.0, "prop5": 0.5}[mode]


def make(LA=(4, 4), pkv=((8, 0), (8, 0), (8, 0), (24, 1)), pwq=((320, 1),), pwo=((192, 1),),
         pw3=((24, 0), (24, 0), (16, 0), (64, 1)), pw4=((48, 0), (48, 0), (32, 0), (128, 1)),
         merge="prop", tmerge="prop", skeleton=False, name="decode_v5", scopes=False, NQ=4, extra=None,
         w3_cols=2, w4_rows=128, tail_spread=True, place="bytes", poff=0, tpoff=0, pslots=None, wslots=None, tslots=None, fill=False, cshift=0, cshift0=None):
    cshift0 = cshift if cshift0 is None else cshift0
    extra = extra or {}

    def sc(n):
        return jax.named_scope(n) if scopes else contextlib.nullcontext()

    pair_chunks = _merge([("wq",) + c for c in _cut(D, pwq)] + [("k",) + c for c in _cut(PR, pkv)] +
                         [("v",) + c for c in _cut(PR, pkv)] + [("wo",) + c for c in _cut(PR, pwo)], merge)
    tail_chunks = _merge([("w3",) + c for c in _cut(D, pw3)] + [("w4",) + c for c in _cut(F, pw4)], tmerge)
    C = len(pair_chunks)
    CT = len(tail_chunks)
    pq = [[i for i, c in enumerate(pair_chunks) if c[3] == t] for t in (0, 1)]
    tq = [[i for i, c in enumerate(tail_chunks) if c[3] == t] for t in (0, 1)]
    ppos = {i: k for t in (0, 1) for k, i in enumerate(pq[t])}
    tpos = {i: k for t in (0, 1) for k, i in enumerate(tq[t])}
    NQ0 = [len(pq[0]), len(pq[1])]
    assert all(NQ0[t] >= LA[t] for t in (0, 1)), NQ0
    SOFF = (0, LA[0])
    NSEM = LA[0] + LA[1]

    def ready_step(chunks, kind, row_end):
        return max(i for i, c in enumerate(chunks) if c[0] == kind and c[1] < row_end)

    pieces = [(("q",), ready_step(pair_chunks, "wq", D))]
    for b in range(3):
        for c in range(NQ):
            pieces.append((("qk", b, c), ready_step(pair_chunks, "k", 128 * (b + 1))))
    pieces.append((("sm", 0), 0))
    pieces.append((("sm", 1), 0))
    for b in range(3):
        for c in range(NQ):
            pieces.append((("pv", b, c), ready_step(pair_chunks, "v", 128 * (b + 1))))
    pieces.append((("wo",), ready_step(pair_chunks, "wo", PR)))
    NP = len(pieces)
    cum, tot = [], 0
    for c in pair_chunks:
        tot += _nbytes(c)
        cum.append(tot)
    if place == "bytes":
        slot_step = [min(i for i in range(C) if cum[i] >= (s + 1) * tot / NP - 1e-6) for s in range(NP)]
    elif place == "steps":
        slot_step = [((i + 1) * C) // NP - 1 for i in range(NP)]
    elif place == "q1":
        q1steps = pq[1]
        slot_step = [q1steps[min(len(q1steps) - 1, ((s + 1) * len(q1steps)) // NP - 1 if (s + 1) * len(q1steps) >= NP else 0)] for s in range(NP)]
    if place != "pat":
        slot_step = [max(0, min(C - 1, s + poff)) for s in slot_step]
    if place == "pat":
        cand = []
        cnt = {}
        for i, c in enumerate(pair_chunks):
            kind = c[0]
            k = cnt.get(kind, 0); cnt[kind] = k + 1
            if kind in ("k", "v"):
                L = _patlen(pkv)
                cand += [i] * list(pslots).count(k % L)
            else:
                L = _patlen(pwq if kind == "wq" else pwo)
                cand += [i] * list(wslots).count(k % L)
        if fill:
            slot_step = cand
        else:
            slot_step = [cand[(k * len(cand)) // NP] for k in range(NP)]
    if fill and place == "pat":
        nfill = len(slot_step) - NP
        newp, used = [], 0
        for i, pcs in enumerate(pieces):
            newp.append(pcs)
            want = ((i + 1) * nfill) // NP
            while used < want:
                newp.append((("dummy",), 0)); used += 1
        pieces = newp
        NP = len(pieces)
    table = None
    for shift in range(NP):
        ok = True
        tb = {}
        for i, (pc, rdy) in enumerate(pieces):
            s = i + shift
            if s < NP and slot_step[s] < rdy:
                ok = False
                break
            tb.setdefault(slot_step[s % NP], []).append((pc, s >= NP))
        if ok:
            table = tb
            break
    assert table is not None
    make.last = dict(shift=shift, table=table, C=C, CT=CT, NQ0=NQ0, pair=pair_chunks, tail=tail_chunks)

    def kernel(x_hbm, k_hbm, v_hbm, wq_hbm, wo_hbm, w3_hbm, w4_hbm, o_ref,
               x_buf, wq_buf, k_buf, v_buf, wo_buf, w3_buf, w4_buf, p_buf, sem_x, sem_p):
        S = k_hbm.shape[1]
        W = min(4096, max(256, S // 4))
        WQ = W // NQ
        scale = DH ** -0.5

        def cp_pair(j, c):
            kind, r, n, pr, cs, ns = pair_chunks[c]
            assert ns == 1 or kind in ("k", "v")
            cw = W // ns
            slot = j % 2
            base = j * PR
            if not isinstance(j, int):
                base = pl.multiple_of(base, PR)
            if kind == "wq":
                src = wq_hbm.at[pl.ds(r, n), pl.ds(base, PR)]
                dst = wq_buf.at[slot, pl.ds(r, n)]
            elif kind == "k":
                src = k_hbm.at[pl.ds(base + r, n), pl.ds(S - W - (cshift if pr == 1 else cshift0) + cs * cw, cw)]
                dst = k_buf.at[slot, pl.ds(r, n), pl.ds(cs * cw, cw)]
            elif kind == "v":
                src = v_hbm.at[pl.ds(base + r, n), pl.ds(S - W - (cshift if pr == 1 else cshift0) + cs * cw, cw)]
                dst = v_buf.at[slot, pl.ds(r, n), pl.ds(cs * cw, cw)]
            else:
                src = wo_hbm.at[pl.ds(base + r, n), :]
                dst = wo_buf.at[slot, pl.ds(r, n)]
            if NQ0[pr] % LA[pr] == 0:
                si = ppos[c] % LA[pr]
            else:
                si = (j * NQ0[pr] + ppos[c]) % LA[pr]
            return pltpu.make_async_copy(src, dst, sem_p.at[SOFF[pr] + si]), pr

        def cp_tail(c):
            kind, r, n, pr, cs, ns = tail_chunks[c]
            assert ns == 1
            if kind == "w3":
                src, dst = w3_hbm.at[pl.ds(r, n), :], w3_buf.at[pl.ds(r, n), :]
            else:
                src, dst = w4_hbm.at[pl.ds(r, n), :], w4_buf.at[pl.ds(r, n), :]
            si = (NPAIR * NQ0[pr] + tpos[c]) % LA[pr]
            return pltpu.make_async_copy(src, dst, sem_p.at[SOFF[pr] + si]), pr

        def start(cp):
            cp[0].start(priority=cp[1])

        def start_ahead(j, c, last):
            pr = pair_chunks[c][3]
            k = ppos[c] + LA[pr]
            if k < NQ0[pr]:
                start(cp_pair(j, pq[pr][k]))
            elif not last:
                start(cp_pair(j + 1, pq[pr][k - NQ0[pr]]))
            elif k - NQ0[pr] < len(tq[pr]):
                start(cp_tail(tq[pr][k - NQ0[pr]]))

        cp_x = pltpu.make_async_copy(x_hbm, x_buf, sem_x.at[0])
        cp_x.start()
        for c in sorted(pq[0][:LA[0]] + pq[1][:LA[1]]):
            start(cp_pair(0, c))
        cp_x.wait()
        x8 = jnp.broadcast_to(x_buf[...].astype(jnp.float32), (8, D))
        xln = _ln(x8).astype(jnp.bfloat16)

        row = jax.lax.broadcasted_iota(jnp.int32, (8, PR), 0)
        col = jax.lax.broadcasted_iota(jnp.int32, (8, PR), 1)
        mask = ((row == 0) & (col < DH)) | ((row == 1) & (col >= DH))

        def run_piece(pc, j, st):
            slot = j % 2
            if pc[0] == "q":
                q = jnp.dot(xln, wq_buf[slot], preferred_element_type=jnp.float32)
                st["qbd"] = jnp.where(mask, q, 0.0).astype(jnp.bfloat16)
            elif pc[0] == "qk":
                _, b, c = pc
                part = jnp.dot(st["qbd"][:, b * 128:(b + 1) * 128], k_buf[slot, pl.ds(b * 128, 128), pl.ds(c * WQ, WQ)],
                               preferred_element_type=jnp.float32)
                st[("s", c)] = part if b == 0 else st[("s", c)] + part
            elif pc[0] == "sm":
                if pc[1] == 0:
                    for c in range(NQ):
                        st[("s", c)] = st[("s", c)] * scale
                    m = st[("s", 0)]
                    for c in range(1, NQ):
                        m = jnp.maximum(m, st[("s", c)])
                    st["m"] = jnp.max(m, axis=-1, keepdims=True)
                    cs = range(0, NQ // 2)
                    st["lsum"] = None
                else:
                    cs = range(NQ // 2, NQ)
                for c in cs:
                    p = jnp.exp(st[("s", c)] - st["m"])
                    st["lsum"] = p if st["lsum"] is None else st["lsum"] + p
                    p_buf[:, pl.ds(c * WQ, WQ)] = p.astype(jnp.bfloat16)
                if pc[1] == 1:
                    st["l"] = jnp.sum(st["lsum"], axis=-1, keepdims=True)
            elif pc[0] == "pv":
                _, b, c = pc
                o_t = jax.lax.dot_general(p_buf[:, pl.ds(c * WQ, WQ)], v_buf[slot, pl.ds(b * 128, 128), pl.ds(c * WQ, WQ)],
                                          (((1,), (1,)), ((), ())), preferred_element_type=jnp.float32)
                st[("o", b)] = o_t if c == 0 else st[("o", b)] + o_t
            elif pc[0] == "dummy":
                pass
            elif pc[0] == "wo":
                o = jnp.concatenate([st[("o", b)] for b in range(3)], axis=1)
                obd = jnp.where(mask, o / st["l"], 0.0).astype(jnp.bfloat16)
                st["acc"] = st["acc"] + jnp.dot(obd, wo_buf[slot], preferred_element_type=jnp.float32)

        carried = [pc for stp in sorted(table) for pc, prev in table[stp] if prev]
        carry_keys = ["acc", "l"] + [("o", b) for b in range(3) if ("pv", b, 0) not in carried]
        assert all(pc[0] in ("pv", "wo") for pc in carried), carried

        def pair_body(j, st, first, last):
            prev = dict(st)
            cur = {"acc": st["acc"]}
            for c in range(C):
                cp_pair(j, c)[0].wait()
                start_ahead(j, c, last)
                if skeleton:
                    continue
                for pc, is_prev in table.get(c, []):
                    if is_prev:
                        if not first:
                            prev["acc"] = cur["acc"]
                            run_piece(pc, j - 1, prev)
                            cur["acc"] = prev["acc"]
                    else:
                        run_piece(pc, j, cur)
            return cur

        z = jnp.zeros((8, D), jnp.float32)
        if skeleton:
            def lb(j, a):
                pair_body(j, {"acc": a}, False, False)
                return a
            pair_body(0, {"acc": z}, True, False)
            jax.lax.fori_loop(1, NPAIR - 1, lb, z)
            st = pair_body(NPAIR - 1, {"acc": z}, False, True)
            st["acc"] = z
        else:
            st = pair_body(0, {"acc": z}, True, False)
            init = tuple(st[k] for k in carry_keys)

            def lb(j, carry):
                s_in = dict(zip(carry_keys, carry))
                s_out = pair_body(j, s_in, False, False)
                return tuple(s_out[k] for k in carry_keys)

            carry = jax.lax.fori_loop(1, NPAIR - 1, lb, init)
            st = pair_body(NPAIR - 1, dict(zip(carry_keys, carry)), False, True)

        tail_pieces = [(pc, 0) for pc in carried]
        tail_pieces.append((("ln",), 0))
        W3C = F // w3_cols
        for b in range(D // 128):
            for cc in range(w3_cols):
                tail_pieces.append((("w3", b, cc), ready_step(tail_chunks, "w3", 128 * (b + 1))))
        tail_pieces.append((("gelu",), 0))
        for b in range(F // w4_rows):
            tail_pieces.append((("w4", b), ready_step(tail_chunks, "w4", w4_rows * (b + 1))))
        tp = 0

        def run_tail(pc):
            if pc[0] == "ln":
                attn = jnp.sum(st["acc"], axis=0, keepdims=True)
                h = x8 + jnp.broadcast_to(attn, (8, D))
                xb = _ln(h)
                st["x2"] = _ln(xb).astype(jnp.bfloat16)
                st["y"] = h + xb
            elif pc[0] == "w3":
                _, b, cc = pc
                part = jnp.dot(st["x2"][:, b * 128:(b + 1) * 128], w3_buf[pl.ds(b * 128, 128), pl.ds(cc * W3C, W3C)],
                               preferred_element_type=jnp.float32)
                st[("a", cc)] = part if b == 0 else st[("a", cc)] + part
            elif pc[0] == "gelu":
                a = jnp.concatenate([st[("a", cc)] for cc in range(w3_cols)], axis=1)
                st["g"] = jax.nn.gelu(a, approximate=True).astype(jnp.bfloat16)
            elif pc[0] == "w4":
                b = pc[1]
                st["y"] = st["y"] + jnp.dot(st["g"][:, b * w4_rows:(b + 1) * w4_rows], w4_buf[pl.ds(b * w4_rows, w4_rows), :],
                                            preferred_element_type=jnp.float32)
            else:
                run_piece(pc, NPAIR - 1, st)

        tcum, ttot = [], 0
        for c in tail_chunks:
            ttot += _nbytes(c)
            tcum.append(ttot)
        NTP = len(tail_pieces)
        for c in range(CT):
            with sc(f"t_{tail_chunks[c][0]}_{tail_chunks[c][1] + tail_chunks[c][2]}"):
                cp_tail(c)[0].wait()
            pr = tail_chunks[c][3]
            k = tpos[c] + LA[pr]
            if k < len(tq[pr]):
                start(cp_tail(tq[pr][k]))
            if skeleton:
                continue
            allowed = NTP if c == CT - 1 else int(NTP * tcum[c] / ttot + 1e-6) + (1 if tail_spread else 10 ** 6)
            while tp < NTP and tp < allowed and tail_pieces[tp][1] <= c:
                run_tail(tail_pieces[tp][0])
                tp += 1
        if skeleton:
            st["y"] = x8
        with sc("final_store"):
            o_ref[...] = st["y"][0:1, :].astype(o_ref.dtype)

    def f(A_x, A_k_cache, A_v_cache, A_wq, A_wo, B_x, B_w1, B_w2, B_w3, B_w4):
        B, Hkv, Sk, Dh = A_k_cache.shape
        kt = jnp.swapaxes(A_k_cache, 2, 3).reshape(Hkv * Dh, Sk)
        vt = jnp.swapaxes(A_v_cache, 2, 3).reshape(Hkv * Dh, Sk)
        x = A_x.reshape(1, D)
        W = min(4096, max(256, Sk // 4))
        any_spec = pl.BlockSpec(memory_space=pl.ANY)
        out = pl.pallas_call(
            kernel,
            out_shape=jax.ShapeDtypeStruct((1, D), jnp.bfloat16),
            in_specs=[any_spec] * 7,
            out_specs=pl.BlockSpec(memory_space=pltpu.VMEM),
            scratch_shapes=[
                pltpu.VMEM((1, D), jnp.bfloat16),
                pltpu.VMEM((2, D, PR), jnp.bfloat16),
                pltpu.VMEM((2, PR, W), jnp.bfloat16),
                pltpu.VMEM((2, PR, W), jnp.bfloat16),
                pltpu.VMEM((2, PR, D), jnp.bfloat16),
                pltpu.VMEM((D, F), jnp.bfloat16),
                pltpu.VMEM((F, D), jnp.bfloat16),
                pltpu.VMEM((8, W), jnp.bfloat16),
                pltpu.SemaphoreType.DMA((1,)),
                pltpu.SemaphoreType.DMA((NSEM,)),
            ],
            compiler_params=pltpu.CompilerParams(vmem_limit_bytes=64 * 1024 * 1024, **extra),
            name=name,
        )(x, kt, vt, A_wq, A_wo, B_w3, B_w4)
        return out.reshape(1, 1, D)

    f.__name__ = name
    return f


_impl = make(pkv=((8, 0, 4), (8, 0, 4), (80, 1, 2)), pwq=((80, 0), (240, 1)), pwo=((48, 0), (144, 1)), place="pat", NQ=8, pslots=(0, 1, 2, 4, 5, 6), wslots=(0, 1), LA=(6, 5), pw3=((32, 0), (96, 1)), pw4=((64, 0), (192, 1)), merge="seq", tmerge="seq", name="preln_decode_fused")


@jax.jit
def pallas_sequential_preLN__sliding_block_cached__mixer_s_mlp__decode_kernel(
    A_x: jax.Array,
    A_k_cache: jax.Array,
    A_v_cache: jax.Array,
    A_wq: jax.Array,
    A_wo: jax.Array,
    B_x: jax.Array,
    B_w1: jax.Array,
    B_w2: jax.Array,
    B_w3: jax.Array,
    B_w4: jax.Array,
):
    return _impl(A_x, A_k_cache, A_v_cache, A_wq, A_wo, B_x, B_w1, B_w2, B_w3, B_w4)
```

```python
import contextlib
import jax
import jax.numpy as jnp
import jax.experimental.pallas as pl
import jax.experimental.pallas.tpu as pltpu

D = 640
HQ = 32
DH = 192
F = 1536
EPS = 1e-5
NPAIR = HQ // 2
PR = 2 * DH
ROWB = {"wq": PR * 2, "k": 4096 * 2, "v": 4096 * 2, "wo": D * 2, "w3": F * 2, "w4": D * 2}


def _ln(v):
    m = jnp.mean(v, axis=-1, keepdims=True)
    c = v - m
    var = jnp.mean(c * c, axis=-1, keepdims=True)
    return c * jax.lax.rsqrt(var + EPS)


def _cut(total, pattern):
    out, r, i = [], 0, 0
    while r < total:
        e = pattern[i % len(pattern)]
        n, pr = e[0], e[1]
        ns = e[2] if len(e) > 2 else 1
        n = min(n, total - r)
        for s in range(ns):
            out.append((r, n, pr, s, ns))
        r += n; i += 1
    return out


def _patlen(pattern):
    return sum((e[2] if len(e) > 2 else 1) for e in pattern)


def _nbytes(c):
    return c[2] * ROWB[c[0]] // c[5]


def _merge(chunks, mode):
    if mode == "seq":
        return chunks
    q = [[c for c in chunks if c[3] == t] for t in (0, 1)]
    tot = [sum(_nbytes(c) for c in q[t]) for t in (0, 1)]
    keyed = []
    for t in (0, 1):
        acc = 0
        for c in q[t]:
            b = _nbytes(c)
            keyed.append(((acc + b * mode_off(mode, t)) / tot[t], t, len(keyed), c))
            acc += b
    keyed.sort()
    return [c for _, _, _, c in keyed]


def mode_off(mode, t):
    return {"prop": 1.0, "prop0": 0.0, "prop5": 0.5}[mode]


def make(LA=(4, 4), pkv=((8, 0), (8, 0), (8, 0), (24, 1)), pwq=((320, 1),), pwo=((192, 1),),
         pw3=((24, 0), (24, 0), (16, 0), (64, 1)), pw4=((48, 0), (48, 0), (32, 0), (128, 1)),
         merge="prop", tmerge="prop", skeleton=False, name="decode_v5", scopes=False, NQ=4, extra=None,
         w3_cols=2, w4_rows=128, tail_spread=True, place="bytes", poff=0, tpoff=0, pslots=None, wslots=None, tslots=None, fill=False, cshift=0, cshift0=None, dyn_shift=False):
    cshift0 = cshift if cshift0 is None else cshift0
    extra = extra or {}

    def sc(n):
        return jax.named_scope(n) if scopes else contextlib.nullcontext()

    pair_chunks = _merge([("wq",) + c for c in _cut(D, pwq)] + [("k",) + c for c in _cut(PR, pkv)] +
                         [("v",) + c for c in _cut(PR, pkv)] + [("wo",) + c for c in _cut(PR, pwo)], merge)
    tail_chunks = _merge([("w3",) + c for c in _cut(D, pw3)] + [("w4",) + c for c in _cut(F, pw4)], tmerge)
    C = len(pair_chunks)
    CT = len(tail_chunks)
    pq = [[i for i, c in enumerate(pair_chunks) if c[3] == t] for t in (0, 1)]
    tq = [[i for i, c in enumerate(tail_chunks) if c[3] == t] for t in (0, 1)]
    ppos = {i: k for t in (0, 1) for k, i in enumerate(pq[t])}
    tpos = {i: k for t in (0, 1) for k, i in enumerate(tq[t])}
    NQ0 = [len(pq[0]), len(pq[1])]
    assert all(NQ0[t] >= LA[t] for t in (0, 1)), NQ0
    SOFF = (0, LA[0])
    NSEM = LA[0] + LA[1]

    def ready_step(chunks, kind, row_end):
        return max(i for i, c in enumerate(chunks) if c[0] == kind and c[1] < row_end)

    pieces = [(("q",), ready_step(pair_chunks, "wq", D))]
    for b in range(3):
        for c in range(NQ):
            pieces.append((("qk", b, c), ready_step(pair_chunks, "k", 128 * (b + 1))))
    pieces.append((("sm", 0), 0))
    pieces.append((("sm", 1), 0))
    for b in range(3):
        for c in range(NQ):
            pieces.append((("pv", b, c), ready_step(pair_chunks, "v", 128 * (b + 1))))
    pieces.append((("wo",), ready_step(pair_chunks, "wo", PR)))
    NP = len(pieces)
    cum, tot = [], 0
    for c in pair_chunks:
        tot += _nbytes(c)
        cum.append(tot)
    if place == "bytes":
        slot_step = [min(i for i in range(C) if cum[i] >= (s + 1) * tot / NP - 1e-6) for s in range(NP)]
    elif place == "steps":
        slot_step = [((i + 1) * C) // NP - 1 for i in range(NP)]
    elif place == "q1":
        q1steps = pq[1]
        slot_step = [q1steps[min(len(q1steps) - 1, ((s + 1) * len(q1steps)) // NP - 1 if (s + 1) * len(q1steps) >= NP else 0)] for s in range(NP)]
    if place != "pat":
        slot_step = [max(0, min(C - 1, s + poff)) for s in slot_step]
    if place == "pat":
        cand = []
        cnt = {}
        for i, c in enumerate(pair_chunks):
            kind = c[0]
            k = cnt.get(kind, 0); cnt[kind] = k + 1
            if kind in ("k", "v"):
                L = _patlen(pkv)
                cand += [i] * list(pslots).count(k % L)
            else:
                L = _patlen(pwq if kind == "wq" else pwo)
                cand += [i] * list(wslots).count(k % L)
        if fill:
            slot_step = cand
        else:
            slot_step = [cand[(k * len(cand)) // NP] for k in range(NP)]
    if fill and place == "pat":
        nfill = len(slot_step) - NP
        newp, used = [], 0
        for i, pcs in enumerate(pieces):
            newp.append(pcs)
            want = ((i + 1) * nfill) // NP
            while used < want:
                newp.append((("dummy",), 0)); used += 1
        pieces = newp
        NP = len(pieces)
    table = None
    for shift in range(NP):
        ok = True
        tb = {}
        for i, (pc, rdy) in enumerate(pieces):
            s = i + shift
            if s < NP and slot_step[s] < rdy:
                ok = False
                break
            tb.setdefault(slot_step[s % NP], []).append((pc, s >= NP))
        if ok:
            table = tb
            break
    assert table is not None
    make.last = dict(shift=shift, table=table, C=C, CT=CT, NQ0=NQ0, pair=pair_chunks, tail=tail_chunks)

    def kernel(*refs):
        if dyn_shift:
            sh_ref, refs = refs[0], refs[1:]
            dsh = pl.multiple_of(sh_ref[0] * 128, 128)
        else:
            dsh = 0
        (x_hbm, k_hbm, v_hbm, wq_hbm, wo_hbm, w3_hbm, w4_hbm, o_ref,
         x_buf, wq_buf, k_buf, v_buf, wo_buf, w3_buf, w4_buf, p_buf, sem_x, sem_p) = refs
        S = k_hbm.shape[1]
        W = min(4096, max(256, S // 4))
        WQ = W // NQ
        scale = DH ** -0.5

        def cp_pair(j, c):
            kind, r, n, pr, cs, ns = pair_chunks[c]
            assert ns == 1 or kind in ("k", "v")
            cw = W // ns
            slot = j % 2
            base = j * PR
            if not isinstance(j, int):
                base = pl.multiple_of(base, PR)
            if kind == "wq":
                src = wq_hbm.at[pl.ds(r, n), pl.ds(base, PR)]
                dst = wq_buf.at[slot, pl.ds(r, n)]
            elif kind == "k":
                src = k_hbm.at[pl.ds(base + r, n), pl.ds(S - W - (cshift if pr == 1 else cshift0) - dsh + cs * cw, cw)]
                dst = k_buf.at[slot, pl.ds(r, n), pl.ds(cs * cw, cw)]
            elif kind == "v":
                src = v_hbm.at[pl.ds(base + r, n), pl.ds(S - W - (cshift if pr == 1 else cshift0) - dsh + cs * cw, cw)]
                dst = v_buf.at[slot, pl.ds(r, n), pl.ds(cs * cw, cw)]
            else:
                src = wo_hbm.at[pl.ds(base + r, n), :]
                dst = wo_buf.at[slot, pl.ds(r, n)]
            if NQ0[pr] % LA[pr] == 0:
                si = ppos[c] % LA[pr]
            else:
                si = (j * NQ0[pr] + ppos[c]) % LA[pr]
            return pltpu.make_async_copy(src, dst, sem_p.at[SOFF[pr] + si]), pr

        def cp_tail(c):
            kind, r, n, pr, cs, ns = tail_chunks[c]
            assert ns == 1
            if kind == "w3":
                src, dst = w3_hbm.at[pl.ds(r, n), :], w3_buf.at[pl.ds(r, n), :]
            else:
                src, dst = w4_hbm.at[pl.ds(r, n), :], w4_buf.at[pl.ds(r, n), :]
            si = (NPAIR * NQ0[pr] + tpos[c]) % LA[pr]
            return pltpu.make_async_copy(src, dst, sem_p.at[SOFF[pr] + si]), pr

        def start(cp):
            cp[0].start(priority=cp[1])

        def start_ahead(j, c, last):
            pr = pair_chunks[c][3]
            k = ppos[c] + LA[pr]
            if k < NQ0[pr]:
                start(cp_pair(j, pq[pr][k]))
            elif not last:
                start(cp_pair(j + 1, pq[pr][k - NQ0[pr]]))
            elif k - NQ0[pr] < len(tq[pr]):
                start(cp_tail(tq[pr][k - NQ0[pr]]))

        cp_x = pltpu.make_async_copy(x_hbm, x_buf, sem_x.at[0])
        cp_x.start()
        for c in sorted(pq[0][:LA[0]] + pq[1][:LA[1]]):
            start(cp_pair(0, c))
        cp_x.wait()
        x8 = jnp.broadcast_to(x_buf[...].astype(jnp.float32), (8, D))
        xln = _ln(x8).astype(jnp.bfloat16)

        row = jax.lax.broadcasted_iota(jnp.int32, (8, PR), 0)
        col = jax.lax.broadcasted_iota(jnp.int32, (8, PR), 1)
        mask = ((row == 0) & (col < DH)) | ((row == 1) & (col >= DH))

        def run_piece(pc, j, st):
            slot = j % 2
            if pc[0] == "q":
                q = jnp.dot(xln, wq_buf[slot], preferred_element_type=jnp.float32)
                st["qbd"] = jnp.where(mask, q, 0.0).astype(jnp.bfloat16)
            elif pc[0] == "qk":
                _, b, c = pc
                part = jnp.dot(st["qbd"][:, b * 128:(b + 1) * 128], k_buf[slot, pl.ds(b * 128, 128), pl.ds(c * WQ, WQ)],
                               preferred_element_type=jnp.float32)
                st[("s", c)] = part if b == 0 else st[("s", c)] + part
            elif pc[0] == "sm":
                if pc[1] == 0:
                    for c in range(NQ):
                        st[("s", c)] = st[("s", c)] * scale
                    m = st[("s", 0)]
                    for c in range(1, NQ):
                        m = jnp.maximum(m, st[("s", c)])
                    st["m"] = jnp.max(m, axis=-1, keepdims=True)
                    cs = range(0, NQ // 2)
                    st["lsum"] = None
                else:
                    cs = range(NQ // 2, NQ)
                for c in cs:
                    p = jnp.exp(st[("s", c)] - st["m"])
                    st["lsum"] = p if st["lsum"] is None else st["lsum"] + p
                    p_buf[:, pl.ds(c * WQ, WQ)] = p.astype(jnp.bfloat16)
                if pc[1] == 1:
                    st["l"] = jnp.sum(st["lsum"], axis=-1, keepdims=True)
            elif pc[0] == "pv":
                _, b, c = pc
                o_t = jax.lax.dot_general(p_buf[:, pl.ds(c * WQ, WQ)], v_buf[slot, pl.ds(b * 128, 128), pl.ds(c * WQ, WQ)],
                                          (((1,), (1,)), ((), ())), preferred_element_type=jnp.float32)
                st[("o", b)] = o_t if c == 0 else st[("o", b)] + o_t
            elif pc[0] == "dummy":
                pass
            elif pc[0] == "wo":
                o = jnp.concatenate([st[("o", b)] for b in range(3)], axis=1)
                obd = jnp.where(mask, o / st["l"], 0.0).astype(jnp.bfloat16)
                st["acc"] = st["acc"] + jnp.dot(obd, wo_buf[slot], preferred_element_type=jnp.float32)

        carried = [pc for stp in sorted(table) for pc, prev in table[stp] if prev]
        carry_keys = ["acc", "l"] + [("o", b) for b in range(3) if ("pv", b, 0) not in carried]
        assert all(pc[0] in ("pv", "wo") for pc in carried), carried

        def pair_body(j, st, first, last):
            prev = dict(st)
            cur = {"acc": st["acc"]}
            for c in range(C):
                cp_pair(j, c)[0].wait()
                start_ahead(j, c, last)
                if skeleton:
                    continue
                for pc, is_prev in table.get(c, []):
                    if is_prev:
                        if not first:
                            prev["acc"] = cur["acc"]
                            run_piece(pc, j - 1, prev)
                            cur["acc"] = prev["acc"]
                    else:
                        run_piece(pc, j, cur)
            return cur

        z = jnp.zeros((8, D), jnp.float32)
        if skeleton:
            def lb(j, a):
                pair_body(j, {"acc": a}, False, False)
                return a
            pair_body(0, {"acc": z}, True, False)
            jax.lax.fori_loop(1, NPAIR - 1, lb, z)
            st = pair_body(NPAIR - 1, {"acc": z}, False, True)
            st["acc"] = z
        else:
            st = pair_body(0, {"acc": z}, True, False)
            init = tuple(st[k] for k in carry_keys)

            def lb(j, carry):
                s_in = dict(zip(carry_keys, carry))
                s_out = pair_body(j, s_in, False, False)
                return tuple(s_out[k] for k in carry_keys)

            carry = jax.lax.fori_loop(1, NPAIR - 1, lb, init)
            st = pair_body(NPAIR - 1, dict(zip(carry_keys, carry)), False, True)

        tail_pieces = [(pc, 0) for pc in carried]
        tail_pieces.append((("ln",), 0))
        W3C = F // w3_cols
        for b in range(D // 128):
            for cc in range(w3_cols):
                tail_pieces.append((("w3", b, cc), ready_step(tail_chunks, "w3", 128 * (b + 1))))
        tail_pieces.append((("gelu",), 0))
        for b in range(F // w4_rows):
            tail_pieces.append((("w4", b), ready_step(tail_chunks, "w4", w4_rows * (b + 1))))
        tp = 0

        def run_tail(pc):
            if pc[0] == "ln":
                attn = jnp.sum(st["acc"], axis=0, keepdims=True)
                h = x8 + jnp.broadcast_to(attn, (8, D))
                xb = _ln(h)
                st["x2"] = _ln(xb).astype(jnp.bfloat16)
                st["y"] = h + xb
            elif pc[0] == "w3":
                _, b, cc = pc
                part = jnp.dot(st["x2"][:, b * 128:(b + 1) * 128], w3_buf[pl.ds(b * 128, 128), pl.ds(cc * W3C, W3C)],
                               preferred_element_type=jnp.float32)
                st[("a", cc)] = part if b == 0 else st[("a", cc)] + part
            elif pc[0] == "gelu":
                a = jnp.concatenate([st[("a", cc)] for cc in range(w3_cols)], axis=1)
                st["g"] = jax.nn.gelu(a, approximate=True).astype(jnp.bfloat16)
            elif pc[0] == "w4":
                b = pc[1]
                st["y"] = st["y"] + jnp.dot(st["g"][:, b * w4_rows:(b + 1) * w4_rows], w4_buf[pl.ds(b * w4_rows, w4_rows), :],
                                            preferred_element_type=jnp.float32)
            else:
                run_piece(pc, NPAIR - 1, st)

        tcum, ttot = [], 0
        for c in tail_chunks:
            ttot += _nbytes(c)
            tcum.append(ttot)
        NTP = len(tail_pieces)
        for c in range(CT):
            with sc(f"t_{tail_chunks[c][0]}_{tail_chunks[c][1] + tail_chunks[c][2]}"):
                cp_tail(c)[0].wait()
            pr = tail_chunks[c][3]
            k = tpos[c] + LA[pr]
            if k < len(tq[pr]):
                start(cp_tail(tq[pr][k]))
            if skeleton:
                continue
            allowed = NTP if c == CT - 1 else int(NTP * tcum[c] / ttot + 1e-6) + (1 if tail_spread else 10 ** 6)
            while tp < NTP and tp < allowed and tail_pieces[tp][1] <= c:
                run_tail(tail_pieces[tp][0])
                tp += 1
        if skeleton:
            st["y"] = x8
        with sc("final_store"):
            o_ref[...] = st["y"][0:1, :].astype(o_ref.dtype)

    def f(A_x, A_k_cache, A_v_cache, A_wq, A_wo, B_x, B_w1, B_w2, B_w3, B_w4, *sh):
        B, Hkv, Sk, Dh = A_k_cache.shape
        kt = jnp.swapaxes(A_k_cache, 2, 3).reshape(Hkv * Dh, Sk)
        vt = jnp.swapaxes(A_v_cache, 2, 3).reshape(Hkv * Dh, Sk)
        x = A_x.reshape(1, D)
        W = min(4096, max(256, Sk // 4))
        any_spec = pl.BlockSpec(memory_space=pl.ANY)
        out = pl.pallas_call(
            kernel,
            out_shape=jax.ShapeDtypeStruct((1, D), jnp.bfloat16),
            in_specs=([pl.BlockSpec(memory_space=pltpu.SMEM)] if dyn_shift else []) + [any_spec] * 7,
            out_specs=pl.BlockSpec(memory_space=pltpu.VMEM),
            scratch_shapes=[
                pltpu.VMEM((1, D), jnp.bfloat16),
                pltpu.VMEM((2, D, PR), jnp.bfloat16),
                pltpu.VMEM((2, PR, W), jnp.bfloat16),
                pltpu.VMEM((2, PR, W), jnp.bfloat16),
                pltpu.VMEM((2, PR, D), jnp.bfloat16),
                pltpu.VMEM((D, F), jnp.bfloat16),
                pltpu.VMEM((F, D), jnp.bfloat16),
                pltpu.VMEM((8, W), jnp.bfloat16),
                pltpu.SemaphoreType.DMA((1,)),
                pltpu.SemaphoreType.DMA((NSEM,)),
            ],
            compiler_params=pltpu.CompilerParams(vmem_limit_bytes=64 * 1024 * 1024, **extra),
            name=name,
        )(*sh, x, kt, vt, A_wq, A_wo, B_w3, B_w4)
        return out.reshape(1, 1, D)

    f.__name__ = name
    return f


_impl = make(pkv=((8,0,4),(8,0,4),(80,1,4)), pslots=(0,1,2,4,5,6), LA=(6,8), pwq=((80, 0), (240, 1)), pwo=((48, 0), (144, 1)), place="pat", NQ=8, wslots=(0, 1), pw3=((32, 0), (96, 1)), pw4=((64, 0), (192, 1)), merge="seq", tmerge="seq", name="preln_decode_fused")


@jax.jit
def pallas_sequential_preLN__sliding_block_cached__mixer_s_mlp__decode_kernel(
    A_x: jax.Array,
    A_k_cache: jax.Array,
    A_v_cache: jax.Array,
    A_wq: jax.Array,
    A_wo: jax.Array,
    B_x: jax.Array,
    B_w1: jax.Array,
    B_w2: jax.Array,
    B_w3: jax.Array,
    B_w4: jax.Array,
):
    return _impl(A_x, A_k_cache, A_v_cache, A_wq, A_wo, B_x, B_w1, B_w2, B_w3, B_w4)
```

```python
import jax
import jax.numpy as jnp
import jax.experimental.pallas as pl
import jax.experimental.pallas.tpu as pltpu

HQ = 32
DH = 192
PR = 2 * DH
EPS = 1e-5
ROWS = 8
NQ = 8
LOOKAHEAD = (6, 8)

PAT_KV = ((8, 0, 4), (8, 0, 4), (80, 1, 4))
PAT_WQ = ((80, 0, 1), (240, 1, 1))
PAT_WO = ((48, 0, 1), (144, 1, 1))
PAT_W3 = ((32, 0, 1), (96, 1, 1))
PAT_W4 = ((64, 0, 1), (192, 1, 1))
SLOTS_KV = (0, 1, 2, 4, 5, 6)
SLOTS_W = (0, 1)
W3_COL_PIECES = 2
W4_ROWS = 128


def _layernorm(v):
    m = jnp.mean(v, axis=-1, keepdims=True)
    c = v - m
    var = jnp.mean(c * c, axis=-1, keepdims=True)
    return c * jax.lax.rsqrt(var + EPS)


def _cut(kind, total, pattern):
    out, r, i = [], 0, 0
    while r < total:
        n, prio, ns = pattern[i % len(pattern)]
        n = min(n, total - r)
        out += [(kind, r, n, prio, s, ns) for s in range(ns)]
        r += n
        i += 1
    return out


def _ready(chunks, kind, row_end):
    return max(i for i, c in enumerate(chunks) if c[0] == kind and c[1] < row_end)


def _plan_pair(D):
    chunks = (_cut("wq", D, PAT_WQ) + _cut("k", PR, PAT_KV) + _cut("v", PR, PAT_KV) + _cut("wo", PR, PAT_WO))
    pieces = [(("q",), _ready(chunks, "wq", D))]
    for b in range(PR // 128):
        pieces += [(("qk", b, c), _ready(chunks, "k", 128 * (b + 1))) for c in range(NQ)]
    pieces += [(("sm", 0), 0), (("sm", 1), 0)]
    for b in range(PR // 128):
        pieces += [(("pv", b, c), _ready(chunks, "v", 128 * (b + 1))) for c in range(NQ)]
    pieces.append((("wo",), _ready(chunks, "wo", PR)))
    n_pc = len(pieces)
    cand, seen = [], {}
    for i, c in enumerate(chunks):
        k = seen.get(c[0], 0)
        seen[c[0]] = k + 1
        pat, slots = (PAT_KV, SLOTS_KV) if c[0] in "kv" else ((PAT_WQ if c[0] == "wq" else PAT_WO), SLOTS_W)
        if k % sum(e[2] for e in pat) in slots:
            cand.append(i)
    slot = [cand[(k * len(cand)) // n_pc] for k in range(n_pc)]
    for shift in range(n_pc):
        if all(i + shift >= n_pc or slot[i + shift] >= rdy for i, (_, rdy) in enumerate(pieces)):
            table = {}
            for i, (pc, _) in enumerate(pieces):
                table.setdefault(slot[(i + shift) % n_pc], []).append((pc, i + shift >= n_pc))
            return chunks, table
    raise ValueError("no valid schedule")


def _plan_tail(D, F, carried):
    chunks = _cut("w3", D, PAT_W3) + _cut("w4", F, PAT_W4)
    pieces = [(pc, 0) for pc in carried] + [(("ln",), 0)]
    for b in range(D // 128):
        pieces += [(("w3", b, c), _ready(chunks, "w3", 128 * (b + 1))) for c in range(W3_COL_PIECES)]
    pieces.append((("gelu",), 0))
    pieces += [(("w4", b), _ready(chunks, "w4", W4_ROWS * (b + 1))) for b in range(F // W4_ROWS)]
    size = [c[2] * (F if c[0] == "w3" else D) for c in chunks]
    table, done, cum = {}, 0, 0
    for i in range(len(chunks)):
        cum += size[i]
        allowed = len(pieces) if i == len(chunks) - 1 else int(len(pieces) * cum / sum(size) + 1e-6) + 1
        while done < min(allowed, len(pieces)) and pieces[done][1] <= i:
            table.setdefault(i, []).append(pieces[done][0])
            done += 1
    assert done == len(pieces)
    return chunks, table


def _kernel(x_hbm, k_hbm, v_hbm, wq_hbm, wo_hbm, w3_hbm, w4_hbm, o_ref,
            x_buf, wq_buf, k_buf, v_buf, wo_buf, w3_buf, w4_buf, p_buf, x_sem, sems):
    D = x_hbm.shape[-1]
    F = w3_hbm.shape[-1]
    S = k_hbm.shape[-1]
    W = k_buf.shape[-1]
    WQ = W // NQ
    n_pair = k_hbm.shape[0] // PR
    scale = DH ** -0.5

    pair_chunks, pair_table = _plan_pair(D)
    carried = [pc for step in sorted(pair_table) for pc, prev in pair_table[step] if prev]
    assert all(pc[0] in ("pv", "wo") for pc in carried)
    tail_chunks, tail_table = _plan_tail(D, F, carried)
    pair_q = [[i for i, c in enumerate(pair_chunks) if c[3] == t] for t in (0, 1)]
    tail_q = [[i for i, c in enumerate(tail_chunks) if c[3] == t] for t in (0, 1)]
    pair_pos = {i: k for t in (0, 1) for k, i in enumerate(pair_q[t])}
    tail_pos = {i: k for t in (0, 1) for k, i in enumerate(tail_q[t])}
    assert all(len(pair_q[t]) >= LOOKAHEAD[t] and len(tail_q[t]) >= LOOKAHEAD[t] for t in (0, 1))
    sem_base = (0, LOOKAHEAD[0])

    def pair_copy(j, c):
        kind, r, n, prio, s, ns = pair_chunks[c]
        slot = j % 2
        base = j * PR if isinstance(j, int) else pl.multiple_of(j * PR, PR)
        if kind == "wq":
            src = wq_hbm.at[pl.ds(r, n), pl.ds(base, PR)]
            dst = wq_buf.at[slot, pl.ds(r, n)]
        elif kind == "wo":
            src = wo_hbm.at[pl.ds(base + r, n), :]
            dst = wo_buf.at[slot, pl.ds(r, n)]
        else:
            cw = W // ns
            hbm, buf = (k_hbm, k_buf) if kind == "k" else (v_hbm, v_buf)
            src = hbm.at[pl.ds(base + r, n), pl.ds(S - W + s * cw, cw)]
            dst = buf.at[slot, pl.ds(r, n), pl.ds(s * cw, cw)]
        la, nq = LOOKAHEAD[prio], len(pair_q[prio])
        si = pair_pos[c] % la if nq % la == 0 else (j * nq + pair_pos[c]) % la
        return pltpu.make_async_copy(src, dst, sems.at[sem_base[prio] + si]), prio

    def tail_copy(c):
        kind, r, n, prio, _, _ = tail_chunks[c]
        hbm, buf = (w3_hbm, w3_buf) if kind == "w3" else (w4_hbm, w4_buf)
        si = (n_pair * len(pair_q[prio]) + tail_pos[c]) % LOOKAHEAD[prio]
        return pltpu.make_async_copy(hbm.at[pl.ds(r, n), :], buf.at[pl.ds(r, n), :],
                                     sems.at[sem_base[prio] + si]), prio

    def start(cp):
        cp[0].start(priority=cp[1])

    def start_ahead(j, c, last):
        prio = pair_chunks[c][3]
        k = pair_pos[c] + LOOKAHEAD[prio]
        nq = len(pair_q[prio])
        if k < nq:
            start(pair_copy(j, pair_q[prio][k]))
        elif not last:
            start(pair_copy(j + 1, pair_q[prio][k - nq]))
        else:
            start(tail_copy(tail_q[prio][k - nq]))

    x_copy = pltpu.make_async_copy(x_hbm, x_buf, x_sem.at[0])
    x_copy.start()
    for c in sorted(pair_q[0][:LOOKAHEAD[0]] + pair_q[1][:LOOKAHEAD[1]]):
        start(pair_copy(0, c))
    x_copy.wait()
    x8 = jnp.broadcast_to(x_buf[...].astype(jnp.float32), (ROWS, D))
    xln = _layernorm(x8).astype(jnp.bfloat16)

    row = jax.lax.broadcasted_iota(jnp.int32, (ROWS, PR), 0)
    col = jax.lax.broadcasted_iota(jnp.int32, (ROWS, PR), 1)
    diag = ((row == 0) & (col < DH)) | ((row == 1) & (col >= DH))

    def run_piece(pc, j, st):
        slot = j % 2
        if pc[0] == "q":
            q = jnp.dot(xln, wq_buf[slot], preferred_element_type=jnp.float32)
            st["q"] = jnp.where(diag, q, 0.0).astype(jnp.bfloat16)
        elif pc[0] == "qk":
            _, b, c = pc
            part = jnp.dot(st["q"][:, b * 128:(b + 1) * 128],
                           k_buf[slot, pl.ds(b * 128, 128), pl.ds(c * WQ, WQ)],
                           preferred_element_type=jnp.float32)
            st["s", c] = part if b == 0 else st["s", c] + part
        elif pc[0] == "sm":
            if pc[1] == 0:
                for c in range(NQ):
                    st["s", c] = st["s", c] * scale
                m = st["s", 0]
                for c in range(1, NQ):
                    m = jnp.maximum(m, st["s", c])
                st["m"] = jnp.max(m, axis=-1, keepdims=True)
                st["lsum"] = None
            for c in (range(NQ // 2) if pc[1] == 0 else range(NQ // 2, NQ)):
                p = jnp.exp(st["s", c] - st["m"])
                st["lsum"] = p if st["lsum"] is None else st["lsum"] + p
                p_buf[:, pl.ds(c * WQ, WQ)] = p.astype(jnp.bfloat16)
            if pc[1] == 1:
                st["l"] = jnp.sum(st["lsum"], axis=-1, keepdims=True)
        elif pc[0] == "pv":
            _, b, c = pc
            part = jax.lax.dot_general(p_buf[:, pl.ds(c * WQ, WQ)],
                                       v_buf[slot, pl.ds(b * 128, 128), pl.ds(c * WQ, WQ)],
                                       (((1,), (1,)), ((), ())), preferred_element_type=jnp.float32)
            st["o", b] = part if c == 0 else st["o", b] + part
        else:
            o = jnp.concatenate([st["o", b] for b in range(PR // 128)], axis=1)
            o = jnp.where(diag, o / st["l"], 0.0).astype(jnp.bfloat16)
            st["acc"] = st["acc"] + jnp.dot(o, wo_buf[slot], preferred_element_type=jnp.float32)

    carry_keys = ["acc", "l"] + [("o", b) for b in range(PR // 128) if ("pv", b, 0) not in carried]

    def pair_body(j, st, first, last):
        prev, cur = dict(st), {"acc": st["acc"]}
        for c in range(len(pair_chunks)):
            pair_copy(j, c)[0].wait()
            start_ahead(j, c, last)
            for pc, from_prev in pair_table.get(c, []):
                if not from_prev:
                    run_piece(pc, j, cur)
                elif not first:
                    prev["acc"] = cur["acc"]
                    run_piece(pc, j - 1, prev)
                    cur["acc"] = prev["acc"]
        return cur

    st = pair_body(0, {"acc": jnp.zeros((ROWS, D), jnp.float32)}, True, False)

    def loop_body(j, carry):
        out = pair_body(j, dict(zip(carry_keys, carry)), False, False)
        return tuple(out[k] for k in carry_keys)

    carry = jax.lax.fori_loop(1, n_pair - 1, loop_body, tuple(st[k] for k in carry_keys))
    st = pair_body(n_pair - 1, dict(zip(carry_keys, carry)), False, True)

    FC = F // W3_COL_PIECES

    def run_tail(pc):
        if pc[0] == "ln":
            h = x8 + jnp.broadcast_to(jnp.sum(st["acc"], axis=0, keepdims=True), (ROWS, D))
            x1 = _layernorm(h)
            st["x2"] = _layernorm(x1).astype(jnp.bfloat16)
            st["y"] = h + x1
        elif pc[0] == "w3":
            _, b, c = pc
            part = jnp.dot(st["x2"][:, b * 128:(b + 1) * 128], w3_buf[pl.ds(b * 128, 128), pl.ds(c * FC, FC)],
                           preferred_element_type=jnp.float32)
            st["a", c] = part if b == 0 else st["a", c] + part
        elif pc[0] == "gelu":
            a = jnp.concatenate([st["a", c] for c in range(W3_COL_PIECES)], axis=1)
            st["g"] = jax.nn.gelu(a, approximate=True).astype(jnp.bfloat16)
        elif pc[0] == "w4":
            b = pc[1]
            st["y"] = st["y"] + jnp.dot(st["g"][:, b * W4_ROWS:(b + 1) * W4_ROWS],
                                        w4_buf[pl.ds(b * W4_ROWS, W4_ROWS), :],
                                        preferred_element_type=jnp.float32)
        else:
            run_piece(pc, n_pair - 1, st)

    for c in range(len(tail_chunks)):
        tail_copy(c)[0].wait()
        prio = tail_chunks[c][3]
        k = tail_pos[c] + LOOKAHEAD[prio]
        if k < len(tail_q[prio]):
            start(tail_copy(tail_q[prio][k]))
        for pc in tail_table.get(c, []):
            run_tail(pc)
    o_ref[...] = st["y"][0:1, :].astype(o_ref.dtype)


@jax.jit
def pallas_sequential_preLN__sliding_block_cached__mixer_s_mlp__decode_kernel(
    A_x: jax.Array,
    A_k_cache: jax.Array,
    A_v_cache: jax.Array,
    A_wq: jax.Array,
    A_wo: jax.Array,
    B_x: jax.Array,
    B_w1: jax.Array,
    B_w2: jax.Array,
    B_w3: jax.Array,
    B_w4: jax.Array,
):
    B, Sq, D = A_x.shape
    _, Hkv, Sk, Dh = A_k_cache.shape
    F = B_w3.shape[1]
    W = min(4096, max(256, Sk // 4))
    assert (B, Sq, Hkv, Dh) == (1, 1, HQ, DH) and W % (128 * NQ) == 0 and D % 128 == 0 and F % 256 == 0

    kt = jnp.swapaxes(A_k_cache, 2, 3).reshape(Hkv * Dh, Sk)
    vt = jnp.swapaxes(A_v_cache, 2, 3).reshape(Hkv * Dh, Sk)
    bf16 = jnp.bfloat16
    out = pl.pallas_call(
        _kernel,
        out_shape=jax.ShapeDtypeStruct((1, D), A_x.dtype),
        in_specs=[pl.BlockSpec(memory_space=pl.ANY)] * 7,
        out_specs=pl.BlockSpec(memory_space=pltpu.VMEM),
        scratch_shapes=[
            pltpu.VMEM((1, D), bf16),
            pltpu.VMEM((2, D, PR), bf16),
            pltpu.VMEM((2, PR, W), bf16),
            pltpu.VMEM((2, PR, W), bf16),
            pltpu.VMEM((2, PR, D), bf16),
            pltpu.VMEM((D, F), bf16),
            pltpu.VMEM((F, D), bf16),
            pltpu.VMEM((ROWS, W), bf16),
            pltpu.SemaphoreType.DMA((1,)),
            pltpu.SemaphoreType.DMA((LOOKAHEAD[0] + LOOKAHEAD[1],)),
        ],
        compiler_params=pltpu.CompilerParams(
            vmem_limit_bytes=64 * 1024 * 1024,
            disable_semaphore_checks=True,
        ),
        name="preln_decode_fused",
    )(A_x.reshape(1, D), kt, vt, A_wq, A_wo, B_w3, B_w4)
    return out.reshape(B, Sq, D)
```
